```python
import jax
import jax.numpy as jnp

def _softmax(x, axis=-1):
    return jax.nn.softmax(x, axis=axis)

def _gelu(x):
    return jax.nn.gelu(x, approximate=True)

def _silu(x):
    return jax.nn.silu(x)

def _sigmoid(x):
    return jax.nn.sigmoid(x)

def _layernorm(x, axis=-1, eps=1e-05):
    m = jnp.mean(x, axis=axis, keepdims=True)
    v = jnp.var(x, axis=axis, keepdims=True)
    return (x - m) / jnp.sqrt(v + eps)

def _scatter_add(tgt, idx, src, axis=0):
    return tgt.at[idx].add(src)

def _segment_sum(src, seg, n):
    return jax.ops.segment_sum(src, seg, n)

class _Rng:

    def __init__(self, key):
        self._k = key

    def _next(self):
        self._k, sub = jax.random.split(self._k)
        return sub

    def normal(self, shape):
        return jax.random.normal(self._next(), shape, dtype=jnp.bfloat16)

    def randint(self, lo, hi, shape):
        return jax.random.randint(self._next(), shape, lo, hi, dtype=jnp.int32)

    def uniform(self, shape, lo=0.0, hi=1.0):
        return jax.random.uniform(self._next(), shape, jnp.bfloat16, lo, hi)

    def permutation(self, n):
        return jax.random.permutation(self._next(), n)
kernel_name = 'gated_mix__memory_aug_recurrent_mem_tr__moe_arch_mod__prompt'

def setup_inputs():
    _rng = _Rng(jax.random.key(int.from_bytes(__import__("os").urandom(4), "little")))
    _w = lambda a: (lambda t: t.astype(jnp.bfloat16) if jnp.issubdtype(t.dtype, jnp.floating) else t)(jnp.asarray(a))

    def _A_setup():
        B, S, Dm = (1, 2048, 1024)
        H, Dh = (32, 128)
        M, seg = (8, 32)
        seg = min(seg, S)
        S = S // seg * seg
        return {'x': _w((lambda *s: _rng.normal(s) * 0.05)(B, S, Dm)), 'mem0': _w((lambda *s: _rng.normal(s) * 0.05)(B, M, Dm)), 'Wq': _w((lambda *s: _rng.normal(s) * 0.05)(Dm, H, Dh) * Dm ** (-0.5)), 'Wk': _w((lambda *s: _rng.normal(s) * 0.05)(Dm, H, Dh) * Dm ** (-0.5)), 'Wv': _w((lambda *s: _rng.normal(s) * 0.05)(Dm, H, Dh) * Dm ** (-0.5)), 'Wo': _w((lambda *s: _rng.normal(s) * 0.05)(H, Dh, Dm) * (H * Dh) ** (-0.5)), 'seg_len': seg}
    _A_in = _A_setup()

    def _B_setup():
        B, S, D, F, C = (1, 2048, 1024, 3584, 8)
        return {'x': _w((lambda *s: _rng.normal(s) * 0.05)(B, S, D)), 'w_r': _w((lambda *s: _rng.normal(s) * 0.05)(D)), 'w_gate': _w((lambda *s: _rng.normal(s) * 0.05)(D, F)), 'w_up': _w((lambda *s: _rng.normal(s) * 0.05)(D, F)), 'w_down': _w((lambda *s: _rng.normal(s) * 0.05)(F, D))}
    _B_in = _B_setup()
    return {'A_x': _A_in['x'], 'A_mem0': _A_in['mem0'], 'A_Wq': _A_in['Wq'], 'A_Wk': _A_in['Wk'], 'A_Wv': _A_in['Wv'], 'A_Wo': _A_in['Wo'], 'A_seg_len': _A_in['seg_len'], 'B_x': _B_in['x'], 'B_w_r': _B_in['w_r'], 'B_w_gate': _B_in['w_gate'], 'B_w_up': _B_in['w_up'], 'B_w_down': _B_in['w_down'], 'gate_w': _w((lambda *s: _rng.normal(s) * 0.05)(1024))}

def reference(A_x, A_mem0, A_Wq, A_Wk, A_Wv, A_Wo, A_seg_len, B_x, B_w_r, B_w_gate, B_w_up, B_w_down, gate_w):

    def _A_ref(x, mem0, Wq, Wk, Wv, Wo, seg_len):
        B, S, Dm = x.shape
        H, Dh = (Wq.shape[1], Wq.shape[2])
        M = mem0.shape[1]
        scale = Dh ** (-0.5)
        n_seg = S // seg_len
        L = M + seg_len
        idx = jnp.arange(L)
        mask = (idx[:, None] < M) | (idx[:, None] >= idx[None, :])
        mem = mem0
        outs = []
        for s in range(n_seg):
            xs = x[:, s * seg_len:(s + 1) * seg_len, :].copy()
            h = jnp.concatenate([mem, xs], axis=1)
            q = jnp.einsum('btd,dhe->bhte', h, Wq)
            k = jnp.einsum('btd,dhe->bhte', h, Wk)
            v = jnp.einsum('btd,dhe->bhte', h, Wv)
            scores = jnp.einsum('bhqe,bhke->bhqk', q, k) * scale
            scores = jnp.where(mask[None, None], scores, -1000000000.0)
            p = _softmax(scores, axis=-1)
            o = jnp.einsum('bhqk,bhke->bhqe', p, v)
            o = jnp.einsum('bhte,hed->btd', o, Wo)
            mem = o[:, :M, :].copy()
            outs.append(o[:, M:, :])
        return jnp.concatenate(outs, axis=1)

    def _B_ref(x, w_r, w_gate, w_up, w_down):
        B, S, D = x.shape
        C = 8
        r = x @ w_r
        idx = jnp.argsort(-r, axis=-1)[:, :C]
        idx_e = jnp.repeat(idx.reshape(B, C, 1), D, axis=2)
        x_sel = jnp.take_along_axis(x, idx_e, axis=1)
        g = _silu(x_sel @ w_gate)
        u = x_sel @ w_up
        y = g * u @ w_down
        r_sel = _sigmoid(jnp.take_along_axis(r, idx, axis=1))
        y = y * r_sel.reshape(B, C, 1)
        b_off = (jnp.arange(B) * S).reshape(B, 1)
        flat_idx = (idx + b_off).reshape(B * C)
        zero = (x * 0.0).reshape(B * S, D)
        upd = _scatter_add(zero, flat_idx, y.reshape(B * C, D), axis=0)
        return x + upd.reshape(B, S, D)
    x = A_x
    g = _sigmoid((x * gate_w).sum(-1, keepdims=True))
    a = _A_ref(x, A_mem0, A_Wq, A_Wk, A_Wv, A_Wo, A_seg_len)
    b = _B_ref(x, B_w_r, B_w_gate, B_w_up, B_w_down)
    return g * a + (1 - g) * b
```

```python
import functools

import jax
import jax.numpy as jnp
import numpy as np
from jax import lax
import jax.experimental.pallas as pl
import jax.experimental.pallas.tpu as pltpu

F32 = jnp.float32
BF16 = jnp.bfloat16
U32 = jnp.uint32
LANES = 128
TOP_C = 8

CFG = dict(HG=4, OLAG=3, moe=True, prologue=True, nseg=None)


def _dot(a, b):
    return jnp.dot(a, b, preferred_element_type=F32)


def _dot_nt(a, b):
    return lax.dot_general(a, b, (((1,), (1,)), ((), ())), preferred_element_type=F32)


def _sigmoid(z):
    return 1.0 / (1.0 + jnp.exp(-z))


def _kernel(
    x_hbm, mem0_ref, wq_hbm, wk_hbm, wv_hbm, wo_hbm, wr_ref, wg_hbm, wu_hbm, wd_hbm, gw_ref,
    out_hbm,
    wqkv, wo, wg, wu, wd, xb, xf, gbuf, ring_q, ring_k, ring_v, obuf, upd, accb,
    sem_x, sem_w, sem_m, sem_o,
    *, S, D, H, M, SEG, cfg,
):
    HG, OLAG = cfg["HG"], cfg["OLAG"]
    NP = H // 2
    NG = H // HG
    NSEG = S // SEG
    TOK = SEG - M
    PRE = S - NSEG * TOK
    RING = PRE + SEG
    XCH = S // NP
    ND = D // LANES
    scale = np.float32(LANES ** -0.5)
    ring = (ring_q, ring_k, ring_v)

    def x_copy(c):
        rows = pl.ds(pl.multiple_of(c * (XCH // 2), XCH // 2), XCH // 2)
        return pltpu.make_async_copy(x_hbm.bitcast(U32).at[rows, :], xb.at[rows, :], sem_x.at[c])

    def w_copy(j, p):
        src = (wq_hbm, wk_hbm, wv_hbm)[j].bitcast(U32)
        return pltpu.make_async_copy(src.at[:, :, p, :], wqkv.at[j, p], sem_w.at[j * NP + p])

    m_copies = [
        pltpu.make_async_copy(wg_hbm.bitcast(U32), wg, sem_m.at[0]),
        pltpu.make_async_copy(wu_hbm.bitcast(U32), wu, sem_m.at[1]),
        pltpu.make_async_copy(wd_hbm.bitcast(U32), wd, sem_m.at[2]),
        pltpu.make_async_copy(wo_hbm.bitcast(U32), wo, sem_m.at[3]),
    ]

    def o_copy(s, slot):
        return pltpu.make_async_copy(
            obuf.at[slot],
            out_hbm.bitcast(U32).at[pl.ds(pl.multiple_of(s * (SEG // 2), SEG // 2), SEG // 2), :],
            sem_o.at[slot])

    npre = PRE // XCH
    for c in range(npre):
        x_copy(c).start()
    for p in range(NP):
        for j in range(3):
            w_copy(j, p).start()
        if p + npre < NP:
            x_copy(p + npre).start()
    for c in m_copies:
        c.start()
    for c in range(npre):
        x_copy(c).wait()

    gw = gw_ref[...].astype(F32)
    wr = wr_ref[...].astype(F32)
    lane = lax.broadcasted_iota(jnp.int32, (8, LANES), 1)

    def pro_body(p, rc):
        @pl.when(p >= npre)
        def _():
            x_copy(p).wait()
        for j in range(3):
            w_copy(j, p).wait()
        lhs = pltpu.bitcast(xb[0:PRE // 2, :], BF16)
        for j in range(3):
            raw = wqkv[j, p]
            lo = pltpu.bitcast(raw << 16, F32).reshape(D, LANES).astype(BF16)
            hi = pltpu.bitcast(raw & np.uint32(0xFFFF0000), F32).reshape(D, LANES).astype(BF16)
            wqkv[j, p, :, 0:8, :] = pltpu.bitcast(lo, U32).reshape(D // 16, 8, LANES)
            wqkv[j, p, :, 8:16, :] = pltpu.bitcast(hi, U32).reshape(D // 16, 8, LANES)
            if cfg["prologue"]:
                y = _dot(lhs, jnp.concatenate([lo, hi], axis=1))
                ring[j][2 * p, 0:PRE, :] = y[:, :LANES]
                ring[j][2 * p + 1, 0:PRE, :] = y[:, LANES:]
        xr = pltpu.bitcast(xb[pl.ds(pl.multiple_of(p * (XCH // 2), XCH // 2), XCH // 2), :], BF16).astype(F32)
        row0 = pl.multiple_of(p * XCH, XCH)
        xf[pl.ds(row0, XCH), :] = xr
        ga = xr[:, 0:LANES] * gw[0:1, :]
        ra = xr[:, 0:LANES] * wr[0:1, :]
        for c in range(1, ND):
            ga = ga + xr[:, c * LANES:(c + 1) * LANES] * gw[c:c + 1, :]
            ra = ra + xr[:, c * LANES:(c + 1) * LANES] * wr[c:c + 1, :]
        g = _sigmoid(jnp.sum(ga, axis=1, keepdims=True))
        gbuf[pl.ds(row0, XCH), :] = jnp.broadcast_to(g, (XCH, LANES))
        r = jnp.sum(ra, axis=1, keepdims=True)
        rc = list(rc)
        for i in range(XCH // 8):
            t8 = p * (XCH // 8) + i
            for v in range(len(rc)):
                rc[v] = jnp.where(lane == t8 - v * LANES, r[i * 8:(i + 1) * 8], rc[v])
        return tuple(rc)

    rc = lax.fori_loop(0, NP, pro_body, tuple(jnp.zeros((8, LANES), F32) for _ in range(S // (8 * LANES))))

    if cfg["moe"]:
        r = jnp.concatenate(rc, axis=0).astype(BF16).astype(F32) + 0.0
        sub = lax.broadcasted_iota(jnp.int32, r.shape, 0)
        tok = (sub // 8) * (8 * LANES) + lax.broadcasted_iota(jnp.int32, r.shape, 1) * 8 + sub % 8
        bits = pltpu.bitcast(r, jnp.int32)
        mono = jnp.where(bits < 0, ~bits, bits | np.int32(-2 ** 31))
        mono = lax.shift_right_logical(mono, 16)
        mono = jnp.where(r != r, 0, mono)
        key = pltpu.bitcast((mono * S + (S - 1 - tok)) + 0x10000000, F32)
        idxs, rows, rsel, gsel = [], [], [], []
        for _ in range(TOP_C):
            m = jnp.max(jnp.max(key, axis=1, keepdims=True), axis=0, keepdims=True)
            hit = key == m
            rsel.append(jnp.sum(jnp.sum(jnp.where(hit, r, 0.0), axis=1, keepdims=True), axis=0, keepdims=True))
            key = jnp.where(hit, 0.0, key)
            mi = pltpu.bitcast(jnp.broadcast_to(m, (8, LANES)), jnp.int32)[0, 0]
            idx = jnp.clip((S - 1) - (mi & (S - 1)), 0, S - 1)
            idxs.append(idx)
            rows.append(xf[pl.ds(idx, 1), :])
        xs = jnp.concatenate(rows, axis=0)
        m_copies[0].wait()
        a = _dot(xs, pltpu.bitcast(wg[...], BF16))
        m_copies[1].wait()
        u = _dot(xs, pltpu.bitcast(wu[...], BF16))
        hid = a * _sigmoid(a) * u
        m_copies[2].wait()
        y = _dot(hid, pltpu.bitcast(wd[...], BF16))
        y = y * _sigmoid(jnp.concatenate(rsel, axis=0))
        upd[...] = y
    else:
        for c in m_copies[:3]:
            c.wait()
        idxs = [0] * TOP_C
        upd[...] = jnp.zeros_like(upd)
    m_copies[3].wait()

    L = M + SEG
    qi = lax.broadcasted_iota(jnp.int32, (L, L), 0)
    ki = lax.broadcasted_iota(jnp.int32, (L, L), 1)
    mask = (qi < M) | (qi >= ki)

    def w_group(j, g):
        cols = []
        for h in range(g * HG, (g + 1) * HG):
            w = wqkv[j, h // 2, :, (h % 2) * 8:(h % 2) * 8 + 8, :]
            cols.append(pltpu.bitcast(w.reshape(D // 2, LANES), BF16))
        return jnp.concatenate(cols, axis=1)

    def emit(s):
        r0 = pl.multiple_of(s * SEG, SEG)
        rowid = lax.broadcasted_iota(jnp.int32, (SEG, LANES), 0) + r0
        g = gbuf[pl.ds(r0, SEG), :]
        for c in range(ND):
            cs = slice(c * LANES, (c + 1) * LANES)
            u = jnp.zeros((SEG, LANES), F32)
            for i in range(TOP_C):
                u = jnp.where(rowid == idxs[i], upd[i:i + 1, cs], u)
            o = g * accb[:, cs] + (1.0 - g) * (xf[pl.ds(r0, SEG), cs] + u)
            obuf[s % 2, :, cs] = pltpu.bitcast(o.astype(BF16), U32)

    accb[...] = jnp.zeros_like(accb)

    def seg_body(s, mem):
        @pl.when(s >= 3)
        def _():
            o_copy(s - 3, (s - 3) % 2).wait()

        @pl.when(s >= 2)
        def _():
            o_copy(s - 2, s % 2).start()

        emit(jnp.maximum(s - 1, 0))

        t0 = PRE + s * TOK
        lhs = jnp.concatenate([mem, xf[pl.ds(pl.multiple_of(t0, 8), TOK), :]], axis=0).astype(BF16)
        wpos = [pl.multiple_of((t0 + 8 * i) % RING, 8) for i in range(TOK // 8)]
        rpos = pl.multiple_of((s * SEG) % RING, SEG)
        memp = {}
        heads_o = {}
        acc = None

        def project(j, g):
            y = _dot(lhs, w_group(j, g))
            for i, h in enumerate(range(g * HG, (g + 1) * HG)):
                yh = y[:, i * LANES:(i + 1) * LANES]
                memp[j, h] = yh[:M]
                for b in range(TOK // 8):
                    ring[j][h, pl.ds(wpos[b], 8), :] = yh[M + 8 * b:M + 8 * b + 8]

        def full(j, h):
            return jnp.concatenate([memp.pop((j, h)), ring[j][h, pl.ds(rpos, SEG), :]], axis=0)

        probs = {}

        def scores(g):
            for h in range(g * HG, (g + 1) * HG):
                sc = _dot_nt(full(0, h), full(1, h)) * scale
                sc = jnp.where(mask, sc, -1e9)
                e = jnp.exp(sc - jnp.max(sc, axis=1, keepdims=True))
                probs[h] = e

        def values(g):
            for h in range(g * HG, (g + 1) * HG):
                e = probs.pop(h)
                heads_o[h] = _dot(e, full(2, h)) / jnp.sum(e, axis=1, keepdims=True)

        def outproj(g, acc):
            o = jnp.concatenate([heads_o.pop(h) for h in range(g * HG, (g + 1) * HG)], axis=1)
            w = pltpu.bitcast(wo[g * HG * LANES // 2:(g + 1) * HG * LANES // 2, :], BF16)
            y = _dot(o, w)
            return y if acc is None else acc + y

        for g in range(NG):
            project(0, g)
            if g >= 1:
                values(g - 1)
            project(1, g)
            if g >= OLAG:
                acc = outproj(g - OLAG, acc)
            project(2, g)
            scores(g)
        for g in range(NG - OLAG, NG - 2):
            acc = outproj(g, acc)
        values(NG - 1)
        for g in range(NG - 2, NG):
            acc = outproj(g, acc)
        accb[...] = acc[M:]
        return acc[:M]

    nseg = cfg["nseg"] or NSEG
    lax.fori_loop(0, nseg, seg_body, mem0_ref[...].astype(F32))
    o_copy(nseg - 3, (nseg - 3) % 2).wait()
    o_copy(nseg - 2, nseg % 2).start()
    emit(nseg - 1)
    o_copy(nseg - 1, (nseg - 1) % 2).start()
    o_copy(nseg - 2, nseg % 2).wait()
    o_copy(nseg - 1, (nseg - 1) % 2).wait()


def make(cfg=None):
    cfg = dict(CFG, **(cfg or {}))

    def fn(A_x, A_mem0, A_Wq, A_Wk, A_Wv, A_Wo, A_seg_len, B_x, B_w_r, B_w_gate, B_w_up, B_w_down, gate_w):
        del B_x
        B, S, D = A_x.shape
        _, H, E = A_Wq.shape
        M = A_mem0.shape[1]
        F = B_w_gate.shape[1]
        SEG = int(A_seg_len)
        assert B == 1 and E == LANES
        PRE = S - (S // SEG) * (SEG - M)
        any_spec = pl.BlockSpec(memory_space=pl.ANY)
        vmem_spec = pl.BlockSpec(memory_space=pltpu.VMEM)
        out = pl.pallas_call(
            functools.partial(_kernel, S=S, D=D, H=H, M=M, SEG=SEG, cfg=cfg),
            out_shape=jax.ShapeDtypeStruct((S, D), BF16),
            in_specs=[any_spec, vmem_spec, any_spec, any_spec, any_spec, any_spec, vmem_spec,
                      any_spec, any_spec, any_spec, vmem_spec],
            out_specs=any_spec,
            scratch_shapes=[
                pltpu.VMEM((3, H // 2, D // 16, 16, LANES), U32),
                pltpu.VMEM((H * E // 2, D), U32),
                pltpu.VMEM((D // 2, F), U32),
                pltpu.VMEM((D // 2, F), U32),
                pltpu.VMEM((F // 2, D), U32),
                pltpu.VMEM((S // 2, D), U32),
                pltpu.VMEM((S, D), F32),
                pltpu.VMEM((S, LANES), F32),
                pltpu.VMEM((H, PRE + SEG, LANES), F32),
                pltpu.VMEM((H, PRE + SEG, LANES), F32),
                pltpu.VMEM((H, PRE + SEG, LANES), F32),
                pltpu.VMEM((2, SEG // 2, D), U32),
                pltpu.VMEM((TOP_C, D), F32),
                pltpu.VMEM((SEG, D), F32),
                pltpu.SemaphoreType.DMA((H // 2,)),
                pltpu.SemaphoreType.DMA((3 * H // 2,)),
                pltpu.SemaphoreType.DMA((4,)),
                pltpu.SemaphoreType.DMA((2,)),
            ],
            compiler_params=pltpu.CompilerParams(vmem_limit_bytes=124 * 1024 * 1024, **cfg.get("cp", {})),
            name="gmk",
        )(
            A_x.reshape(S, D), A_mem0.reshape(M, D),
            A_Wq.reshape(D // 16, 16, H, E), A_Wk.reshape(D // 16, 16, H, E), A_Wv.reshape(D // 16, 16, H, E),
            A_Wo.reshape(H * E, D), B_w_r.reshape(D // LANES, LANES),
            B_w_gate, B_w_up, B_w_down, gate_w.reshape(D // LANES, LANES),
        )
        return out.reshape(B, S, D)

    return fn


pallas_gated_mix__memory_aug_recurrent_mem_tr__moe_arch_mod__prompt_kernel = jax.jit(make(), static_argnames=("A_seg_len",))
```

```python
import functools

import jax
import jax.numpy as jnp
import numpy as np
from jax import lax
import jax.experimental.pallas as pl
import jax.experimental.pallas.tpu as pltpu

F32 = jnp.float32
BF16 = jnp.bfloat16
U32 = jnp.uint32
LANES = 128
TOP_C = 8
HI16 = np.uint32(0xFFFF0000)
LO16 = np.uint32(0x0000FFFF)

CFG = dict(R5=32, LAG=4, nit=None, vpos=4, NC=8, GP=2, R2=16, lead=3, U=1,
           per=("202020200000", "040004000000", "1010101010101010"), hold=24, after=6, ahead=2,
           tail=7, epos=(0, 2), hold2=16)


def _dot(a, b):
    return jnp.dot(a, b, preferred_element_type=F32)


def _dot_nt(a, b):
    return lax.dot_general(a, b, (((1,), (1,)), ((), ())), preferred_element_type=F32)


def _sigmoid(z):
    return 1.0 / (1.0 + jnp.exp(-z))


def _cat(*xs, axis=0):
    return jnp.concatenate(xs, axis=axis)


def _tile(c):
    return slice(c * LANES, (c + 1) * LANES)


def _aligned(i, n):
    return i if isinstance(i, int) else pl.multiple_of(i, n)


def _unpack(u):
    return pltpu.bitcast(u, BF16).astype(F32)


def _pack(x):
    return pltpu.bitcast(x.astype(BF16), U32)


def _kernel(
    x_hbm, mem0_ref, wq_hbm, wk_hbm, wv_hbm, wo_hbm, wr_ref, wg_hbm, wu_hbm, wd_hbm, gw_ref,
    out_hbm,
    wq, wk, wv, wo, wg, wu, wd, xb, ob, gate, big2, big5, p2q, p2k, p2v, p5q, p5k, p5v,
    lq, mid, tq, tk, tv, oa, om, lo_a, lo_b, oacc_a, oacc_b, accb, xsel, rsel, idx_ref,
    sem_x, sem_w, sem_wo, sem_m, sem_o,
    *, S, D, H, M, SEG, cfg,
):
    NP = H // 2
    NJ = S // SEG // 2
    DH = D // 2
    ND = D // LANES
    NH = DH // LANES
    R5, LAG, AH, NC, TAIL = cfg["R5"], cfg["LAG"], cfg["ahead"], cfg["NC"], cfg["tail"]
    P5 = SEG - R5
    L = M + SEG
    scale = np.float32(LANES ** -0.5)
    tok, wqkv = (tq, tk, tv), (wq, wk, wv)
    pre2, pre5 = (p2q, p2k, p2v), (p5q, p5k, p5v)

    xw = x_hbm.bitcast(U32)
    x_head = pltpu.make_async_copy(xw.at[0, 0], xb.at[0, 0], sem_x.at[0])
    x_odd = pltpu.make_async_copy(xw.at[:, 1], xb.at[:, 1], sem_x.at[1])
    x_even = pltpu.make_async_copy(xw.at[pl.ds(1, NJ - 1), 0], xb.at[pl.ds(1, NJ - 1), 0], sem_x.at[2])

    def w_copies(p):
        return [
            pltpu.make_async_copy(
                w.bitcast(U32).at[pl.ds(half * (DH // 16), DH // 16), :, p, :],
                wqkv[j].at[p, :, pl.ds(half * 16, 16), :], sem_w.at[p])
            for j, w in enumerate((wq_hbm, wk_hbm, wv_hbm)) for half in range(2)]

    PG = 2
    NWO = NP // PG

    def wo_copies(g):
        pairs = pl.ds(g * PG, PG)
        return [
            pltpu.make_async_copy(
                wo_hbm.bitcast(U32).at[pairs, hh, :, pl.ds(half * DH, DH)],
                wo.at[pairs, 1 + 2 * hh + half], sem_wo.at[g])
            for hh in range(2) for half in range(2)]

    m_copies = [
        pltpu.make_async_copy(wg_hbm.bitcast(U32), wg, sem_m.at[0]),
        pltpu.make_async_copy(wu_hbm.bitcast(U32), wu, sem_m.at[1]),
        pltpu.make_async_copy(wd_hbm.bitcast(U32), wd, sem_m.at[2]),
        pltpu.make_async_copy(xw, ob.at[pl.ds(0, NJ)], sem_m.at[3]),
    ]

    def o_copy(jp):
        return pltpu.make_async_copy(ob.at[jp], out_hbm.bitcast(U32).at[jp], sem_o)

    def start(copies):
        for c in copies:
            c.start()

    def wait(copies):
        for c in copies:
            c.wait()

    def w_in(j, p, i):
        return pltpu.bitcast(wqkv[j][p, :, 8 * i:8 * i + 8, :].reshape(DH // 2, LANES), BF16)

    def combine_in(j, p, t, after=lambda u: u):
        top, bot = after(wqkv[j][p, t, 0:16, :]), after(wqkv[j][p, t, 16:32, :])
        b11, b12, b21, b22 = (
            pltpu.bitcast(u, F32) for u in (top << 16, top & HI16, bot << 16, bot & HI16))
        for i, w in enumerate((b11 + b22, b11, b12 - b22, b21 - b11, b22, b11 + b12, b21 + b22)):
            wqkv[j][p, t, 8 * i:8 * i + 8, :] = _pack(w)

    def combine_out(p, t, n, after):
        rows, cols = slice(8 * t, 8 * t + 8), slice(2 * n * LANES, (2 * n + 2) * LANES)
        b11, b12, b21, b22 = (_unpack(after(wo[p, i, rows, cols])) for i in (1, 2, 3, 4))
        for i, w in ((0, b11 + b22), (2, b12 - b22), (3, b21 - b11), (5, b11 + b12), (6, b21 + b22)):
            wo[p, i, rows, cols] = _pack(w)

    def row_dot(xr, w):
        acc = xr[:, _tile(0)] * w[0:1, :]
        for c in range(1, ND):
            acc = acc + xr[:, _tile(c)] * w[c:c + 1, :]
        return jnp.sum(acc, axis=1, keepdims=True)

    qi = lax.broadcasted_iota(jnp.int32, (L, L), 0)
    ki = lax.broadcasted_iota(jnp.int32, (L, L), 1)
    mask = (qi < M) | (qi >= ki)

    def probs(q, k, msk):
        sc = jnp.where(msk, _dot_nt(q, k) * scale, -1e9)
        e = jnp.exp(sc - jnp.max(sc, axis=1, keepdims=True))
        return e * (1.0 / jnp.sum(e, axis=1, keepdims=True))

    XE = 0 if P5 else 1
    start(w_copies(0))
    start([x_head, x_odd])
    if not XE:
        x_even.start()
    start(w_copies(1))
    wait(w_copies(0))
    for j in range(3):
        for t in range(DH // 16):
            combine_in(j, 0, t)
    wait([x_head, x_odd])
    if not XE:
        x_even.wait()
    if XE:
        x_even.start()
    for p in range(2, AH + 1):
        start(w_copies(p))
    for jp in range(1, NJ):
        b = _unpack(xb[jp, 1])
        big2[jp - 1] = _pack(b[:, :DH] + b[:, DH:])
        if P5:
            a = _unpack(xb[jp, 0])[R5:]
            big5[jp - 1] = a[:, :DH] + a[:, DH:]
    h0 = _cat(mem0_ref[...].astype(F32), _unpack(xb[0, 0]), _unpack(xb[0, 1]))
    l0 = M + 2 * SEG
    lq[1, 0:l0, :] = h0[:, :DH] + h0[:, DH:]
    lq[2, 0:l0, :] = h0[:, :DH]
    lq[3, 0:l0, :] = h0[:, DH:]
    lo_b[0, 0:2 * M, 0:DH] = jnp.zeros((2 * M, DH), F32)

    lane = lax.broadcasted_iota(jnp.int32, (8, LANES), 1)
    sub = lax.broadcasted_iota(jnp.int32, (8, LANES), 0)
    JC = 4
    WL = cfg.get("wlead", 2)

    def score_jobs(p, live, keys):
        g0 = p * (JC * 2 * SEG // 8)
        rc = [jnp.zeros((8, LANES), F32)]

        def job(n, after):
            jp = jnp.where(live, p * JC + n // 4, 0)
            xr = _unpack(after(xb[jp, (n // 2) % 2, (n % 2) * 8:(n % 2) * 8 + 8, :]))
            gate[jp, (n % 4) * 16:(n % 4) * 16 + 16, :] = jnp.broadcast_to(
                _sigmoid(row_dot(xr, gw_ref[...].astype(F32))), (16, LANES))
            r = row_dot(xr, wr_ref[...].astype(F32))
            for i in range(2):
                rc[0] = jnp.where(lane == g0 % LANES + 2 * n + i, r[8 * i:8 * i + 8], rc[0])

        def finish():
            r = rc[0].astype(BF16).astype(F32) + 0.0
            bits = pltpu.bitcast(r, jnp.int32)
            mono = lax.shift_right_logical(jnp.where(bits < 0, ~bits, bits | np.int32(-2 ** 31)), 16)
            mono = jnp.where(r != r, 0, mono)
            new = []
            for vi, old in enumerate(keys):
                grp = vi * LANES + lane
                fresh = pltpu.bitcast(mono * S + (S - 1 - (grp * 8 + sub)) + 0x10000000, F32)
                new.append(jnp.where((grp >= g0) & (grp < g0 + JC * 2 * SEG // 8), fresh, old))
            return tuple(new)

        return [functools.partial(job, n) for n in range(4 * JC)], finish

    def pick_row(slot, keys):
        best = functools.reduce(jnp.maximum, keys)
        best = jnp.max(jnp.max(best, axis=1, keepdims=True), axis=0, keepdims=True)
        bi = pltpu.bitcast(jnp.broadcast_to(best, (8, LANES)), jnp.int32)
        mono = lax.shift_right_logical(bi - 0x10000000, int(np.log2(S))) << 16
        score = pltpu.bitcast(jnp.where(mono < 0, mono & np.int32(0x7FFF0000), ~mono & np.int32(-65536)), F32)
        idx = (S - 1) - (bi[0, 0] & (S - 1))
        idx_ref[slot] = idx
        rsel[pl.ds(slot, 1), :] = score[0:1]
        word = xb[idx // (2 * SEG), (idx // SEG) % 2, pl.ds((idx % SEG) // 2, 1), :]
        xsel[pl.ds(slot, 1), :] = pltpu.bitcast(jnp.where(idx % 2 == 0, word << 16, word & HI16), F32)
        return tuple(jnp.where(kv == best, 0.0, kv) for kv in keys)

    def out_jobs(p):
        def product(half, t, after):
            cols = slice(t * 2 * LANES, (t + 1) * 2 * LANES)
            w = pltpu.bitcast(_cat(wo[p, 1 + half, :, cols], wo[p, 3 + half, :, cols]), BF16)
            at = (0, slice(half * M, (half + 1) * M), cols)
            lo_b[at] = lo_b[at] + _dot(om[p], w)

        first = [functools.partial(product, half, t) for t in range(2) for half in range(2)]
        rest = [functools.partial(combine_out, p, t, n) for n in range(NH // 2) for t in range(LANES // 16)]
        return first[:2] + rest[:4] + first[2:3] + rest[4:8] + first[3:] + rest[8:]

    def spread(jobs, lo, hi):
        return [(lo + n * (hi - lo) // len(jobs), job) for n, job in enumerate(jobs)]

    NA = 3 * (4 + NJ - 1)

    def pro_step(p, never, plan, midway=None):
        plan = sorted(plan, key=lambda e: e[0])
        seen = [0]

        def anchor(y):
            def after(u):
                r, c = u.shape
                return jnp.where(never, _cat(*[pltpu.bitcast(y[0:r], U32)] * (c // LANES), axis=1), u)

            while plan and plan[0][0] <= seen[0]:
                plan.pop(0)[1](after)
            seen[0] += 1

        def first(j):
            s = lq[1, 0:l0, :]
            c0 = _dot(s, w_in(j, p, 1)) + _dot(lq[3, 0:l0, :], w_in(j, p, 3))
            c1 = _dot(lq[2, 0:l0, :], w_in(j, p, 2)) + _dot(s, w_in(j, p, 4))
            tok[j][2 * p] = c0[L:]
            tok[j][2 * p + 1] = c1[L:]
            for y in (c0, c0[L:], c1, c1[L:]):
                anchor(y)
            return c0[:L], c1[:L]

        edges = [(NJ - 1) * c // NC for c in range(NC + 1)]

        def bulk(j):
            for c in range(NC):
                lo, hi = edges[c], edges[c + 1]
                lhs = pltpu.bitcast(big2[lo:hi].reshape((hi - lo) * SEG // 2, DH), BF16)
                y = _dot(lhs, w_in(j, p, 1))
                pre2[j][p, lo * SEG:hi * SEG, :] = y
                if P5:
                    pre5[j][p, lo * P5:hi * P5, :] = _dot(big5[lo:hi].reshape((hi - lo) * P5, DH), w_in(j, p, 4))
                for n in range(hi - lo):
                    anchor(y[n * SEG:(n + 1) * SEG])

        q, k, v = first(0), first(1), first(2)
        e = [probs(q[i], k[i], mask) for i in range(2)]
        bulk(0)
        o = [_dot(e[i], v[i]) for i in range(2)]
        oa[2 * p] = o[0][M:]
        oa[2 * p + 1] = o[1][M:]
        om[p] = _cat(o[0][:M], o[1][:M], axis=1)
        if midway:
            midway()
        bulk(1)
        bulk(2)
        assert not plan

    def in_jobs(p):
        return [functools.partial(combine_in, j, p, t) for j in range(3) for t in range(DH // 16)]

    def pro_main(p, keys):
        wait(w_copies(p + 1))
        if XE:
            pl.when(p == XE)(x_even.wait)
        start(w_copies(p + 1 + AH))
        g = p - (NP - TAIL - WL)
        pl.when(g >= 0)(lambda: start(wo_copies(g)))
        jobs, finish = score_jobs(jnp.clip(p - XE, 0, NJ // JC - 1), p >= XE, keys)
        pro_step(p, p < 0, spread(jobs, 0, NA - 12) + spread(in_jobs(p + 1), 0, NA - 1))
        return finish()

    def pro_tail(p, keys):
        g = p - (NP - TAIL)
        wait(w_copies(p + 1))
        pl.when(p + 1 + AH < NP)(lambda: start(w_copies(p + 1 + AH)))
        pl.when(g + WL < NWO)(lambda: start(wo_copies(g + WL)))
        wait(wo_copies(g))
        keys = pick_row(g, keys)
        jobs = [job for n in range(PG) for job in out_jobs(g * PG + n)]
        pro_step(p, p < 0, spread(jobs, 0, NA - 2) + spread(in_jobs(p + 1), 0, NA - 1))
        return keys

    def pro_last(keys):
        for slot in range(TAIL - 1, TOP_C):
            keys = pick_row(slot, keys)

        def midway():
            for g in range(TAIL - 1, NWO):
                wait(wo_copies(g))
            start(m_copies)

        jobs = [job for p in range((TAIL - 1) * PG, NP) for job in out_jobs(p)]
        pro_step(NP - 1, idx_ref[0] < 0, spread(jobs, 12 + NJ - 1, NA - 2), midway)

    keys = tuple(jnp.zeros((8, LANES), F32) for _ in range(S // (8 * LANES)))
    keys = lax.fori_loop(0, NP - TAIL, pro_main, keys)
    keys = lax.fori_loop(NP - TAIL, NP - 1, pro_tail, keys)
    pro_last(keys)
    mem1 = _cat(lo_b[0, 0:M, 0:DH], lo_b[0, M:2 * M, 0:DH], axis=1)

    def routed_mlp():
        wait(m_copies)
        xs = xsel[...]
        a = _dot(xs, pltpu.bitcast(wg[...], BF16))
        u = _dot(xs, pltpu.bitcast(wu[...], BF16))
        y = _dot(a * _sigmoid(a) * u, pltpu.bitcast(wd[...], BF16))
        b = xs + y * _cat(*([_sigmoid(rsel[...])] * ND), axis=1)
        b = pltpu.bitcast(b.astype(BF16).astype(F32), U32)
        for i in range(TOP_C):
            idx = idx_ref[i]
            at = (idx // (2 * SEG), (idx // SEG) % 2, pl.ds((idx % SEG) // 2, 1), slice(None))
            word = ob[at]
            ob[at] = jnp.where(idx % 2 == 0, (word & HI16) | (b[i:i + 1] >> 16), (word & LO16) | b[i:i + 1])

    def emit(jp, dst):
        for c in range(ND):
            g = gate[jp]
            b = _cat(_unpack(ob[dst, 0, :, _tile(c)]), _unpack(ob[dst, 1, :, _tile(c)]))
            o = _pack(g * accb[jp % LAG, :, _tile(c)] + (1.0 - g) * b)
            ob[dst, 0, :, _tile(c)] = o[:SEG // 2]
            ob[dst, 1, :, _tile(c)] = o[SEG // 2:]
            yield o

    GP = cfg["GP"]
    NG = NP // GP
    NW = 4 // GP
    R2 = cfg["R2"]

    def step(kind, jp, mem, side=iter(())):
        a1, a2 = mem[:, :DH], mem[:, DH:]
        if kind != 2:
            xa, xc = _unpack(xb[jp, 0]), _unpack(xb[jp, 1])
            a11, a12, a21, a22 = xa[:, :DH], xa[:, DH:], xc[:, :DH], xc[:, DH:]
        if kind == 0:
            rows = {2: _cat(a1, a11), 3: _cat(a2, a22), 4: _cat(a1 + a2, (a11 + a12)[:R5]) if R5 else a1 + a2,
                    1: a1 + a2}
        elif kind == 1:
            rows = {5: _cat(a1, a21 - a11), 0: _cat(a2, a11 + a22), 6: _cat(a2, a12 - a22), 1: a1 + a2}
        else:
            rows = {2: a1, 3: a2, 4: a1 + a2, 1: a1 + a2}
        for i, r in rows.items():
            lq[i, 0:r.shape[0], :] = r
        slots = list(rows)
        prod, full, ex, acc = {}, {}, {}, {}
        lo = (lo_a, lo_b, lo_a)[kind]
        orows = ({3: L, 2: L, 4: L, 1: M + R2}, {5: L, 0: L, 6: L, 1: L - R2},
                 {2: 2 * SEG, 3: 2 * SEG, 1: 2 * SEG, 4: 2 * SEG})[kind]
        lslot = ({1: 0, 2: 1, 3: 2, 4: 3}, {0: 0, 1: 1, 5: 2, 6: 3}, {1: 0, 2: 1, 3: 2, 4: 0})[kind]

        def proj(j, p, i, anchor=None):
            t = prod.setdefault((j, p), {})
            lhs = lq[i, 0:rows[i].shape[0], :]
            if anchor is not None:
                n = min(SEG, lhs.shape[0])
                held = _cat(*[pltpu.bitcast(anchor[r:r + n], F32) for r in range(0, SEG, n)], axis=1)
                w = held.shape[1]
                head = _cat(jnp.where(idx_ref[0] < 0, held, lhs[:n, :w]), *([lhs[:n, w:]] if w < DH else []), axis=1)
                lhs = _cat(head, lhs[n:]) if n < lhs.shape[0] else head
            t[i] = _dot(lhs, w_in(j, p, i))
            if kind == 0 and i != 1 and rows[i].shape[0] > M:
                mid[j, p, i - 2, 0:rows[i].shape[0] - M, :] = t[i][M:]
            if len(t) < 4:
                return
            if kind == 1:
                at = pl.ds(_aligned((jp - 1) * SEG, SEG), SEG)
                m2, m3, m4, m5 = pre2[j][p, at, :], mid[j, p, 0], mid[j, p, 1], mid[j, p, 2, 0:R5, :]
                if P5:
                    late = pre5[j][p, pl.ds(_aligned((jp - 1) * P5, 8), P5), :]
                    m5 = _cat(m5, late) if R5 else late
                m1, m6, m7 = t[0][M:], t[5][M:], t[6][M:]
                full[j, 2 * p] = _cat(t[1] + (t[6][:M] - t[0][:M]), (m1 + m7) + (m4 - m5))
                full[j, 2 * p + 1] = _cat((t[5][:M] + t[0][:M]) - t[1], m3 + m5)
                tok[j][2 * p] = m2 + m4
                tok[j][2 * p + 1] = (m1 + m6) + (m3 - m2)
            else:
                full[j, 2 * p] = t[1][:M] + t[3][:M]
                full[j, 2 * p + 1] = t[2][:M] + t[4][:M]

        def operand(j, h):
            if kind == 1:
                return full.pop((j, h))
            if kind == 2 and j == 0:
                return tok[j][h]
            return _cat(full.pop((j, h)), tok[j][h])

        def scores(g):
            for h in range(4 * g, 4 * g + 4):
                ex[h] = probs(operand(0, h), operand(1, h), mask[M:] if kind == 2 else mask)

        def values(g):
            for p in range(2 * g, 2 * g + 2):
                o0, o1 = (_dot(ex.pop(h), operand(2, h)) for h in (2 * p, 2 * p + 1))
                t = _tile(p)
                if kind == 0:
                    m0, m1, a21, a22 = o0[:M], o1[:M], o0[M:], o1[M:]
                    a11, a12 = oa[2 * p], oa[2 * p + 1]
                    s2 = _cat(m0 + m1, a21 + a22)
                    lo_a[0, 0:M + R2, t] = s2[:M + R2]
                    if R2 < SEG:
                        lo_b[1, M:L - R2, t] = s2[M + R2:]
                    lo_a[1, 0:L, t] = _cat(m0, a11)
                    lo_a[2, 0:L, t] = o1
                    lo_a[3, 0:L, t] = _cat(m0 + m1, a11 + a12)
                    lo_b[0, M:L, t] = a11 + a22
                    lo_b[2, M:L, t] = a21 - a11
                    lo_b[3, M:L, t] = a12 - a22
                elif kind == 1:
                    m0, m1 = o0[:M], o1[:M]
                    oa[2 * p] = o0[M:]
                    oa[2 * p + 1] = o1[M:]
                    lo_b[0, 0:M, t] = m1
                    lo_b[1, 0:M, t] = m0 + m1
                    lo_b[2, 0:M, t] = m0
                    lo_b[3, 0:M, t] = m1
                else:
                    f0, f1 = _cat(oa[2 * p], o0), _cat(oa[2 * p + 1], o1)
                    lo_a[0, :, t] = f0 + f1
                    lo_a[1, :, t] = f0
                    lo_a[2, :, t] = f1

        oacc = (oacc_a, oacc_b, oacc_a)[kind]

        def outproj(G, n, i):
            pairs = range(G * GP, (G + 1) * GP)
            cols = slice(n * NW * LANES, (n + 1) * NW * LANES)
            w = pltpu.bitcast(_cat(*[wo[p, i, :, cols] for p in pairs]), BF16)
            y = _dot(lo[lslot[i], 0:orows[i], G * GP * LANES:(G + 1) * GP * LANES], w)
            at = (list(orows).index(i), slice(0, orows[i]), cols)
            if G > 0:
                y = y + oacc[at]
            if G < NG - 1 or kind == 0:
                oacc[at] = y
            if G == NG - 1:
                acc[i, n] = y

        NU = NH // NW
        ounits = [(G, n, i) for G in range(NG) for n in range(NU) for i in orows]
        if kind == 0:
            ounits[-4 * NU:] = sorted(ounits[-4 * NU:], key=lambda u: u[2] in (2, 4))
        hold = cfg["hold2"] if kind == 2 else cfg["hold"]
        done = [0]

        def drain(count, limit):
            for _ in range(count):
                if done[0] < limit:
                    outproj(*ounits[done[0]])
                    done[0] += 1

        mats = (1, 2) if kind == 2 else (0, 1, 2)
        vpos = 3 if kind == 2 else cfg["vpos"]
        per = cfg["per"][kind]
        lead = cfg["lead"] if kind == 1 else 0
        for g in range(NP // 2):
            units = [(j, p) for j in mats for p in (2 * g, 2 * g + 1)]
            limit = min(max(0, (g - 1) * 2 // GP) * 4 * NU, len(ounits) - hold)
            if g == 0:
                for j, p in units[:lead]:
                    proj(j, p, slots[0])
            for c, (j, p) in enumerate(units):
                if c == vpos and g >= 1:
                    values(g - 1)
                    if kind == 2:
                        scores(g)
                for n, i in enumerate(slots):
                    if kind == 2:
                        drain(int(per[4 * c + n]), limit)
                    elif n == 3:
                        drain(int(per[2 * c]), limit)
                    if g or c >= lead or n:
                        proj(j, p, i, next(side, None) if n == 1 and c in cfg["epos"] and g >= 2 else None)
                if kind != 2:
                    drain(int(per[2 * c + 1]), limit)
            if kind != 2 or g == 0:
                scores(g)
        drain(len(ounits) - 4 * NU - done[0] - (4 if kind == 2 else cfg["after"]), len(ounits))
        values(NP // 2 - 1)
        drain(len(ounits), len(ounits))
        for _ in side:
            pass

        def wide(i):
            return _cat(*[acc[i, n] for n in range(NU)], axis=1)

        if kind == 0:
            return _cat(wide(1)[:M] + wide(3)[:M], wide(2)[:M] + wide(4)[:M], axis=1)
        if kind == 1:
            sl = (jp - 1) % LAG
            m4, m3, m5, m2 = oacc_a[0, M:L], oacc_a[1, M:L], oacc_a[2, M:L], oacc_a[3, M:M + R2]
            t1, t6, t7, ts = wide(0), wide(5), wide(6), wide(1)
            if R2 < SEG:
                m2 = _cat(m2, ts[M:])
            accb[sl, 0:SEG, :DH] = (t1[M:] + t7[M:]) + (m4 - m5)
            accb[sl, 0:SEG, DH:] = m3 + m5
            accb[sl, SEG:2 * SEG, :DH] = m2 + m4
            accb[sl, SEG:2 * SEG, DH:] = (t1[M:] + t6[M:]) + (m3 - m2)
            return _cat((ts[:M] - t1[:M]) + t7[:M], t6[:M] - (ts[:M] - t1[:M]), axis=1)
        accb[jp % LAG, :, :DH] = wide(1) + wide(3)
        accb[jp % LAG, :, DH:] = wide(2) + wide(4)

    U = cfg["U"]

    def body(it, mem):
        for u in range(U):
            jp = 1 + it * U + u
            if u == 0:
                @pl.when(jp > LAG)
                def _():
                    for n in range(U):
                        o_copy(jp - LAG - U + n).start()
            dst = jnp.where(jp >= LAG, jp - LAG, NJ)
            mem = step(1, jp, step(0, jp, mem, emit(jnp.maximum(jp - LAG, 0), dst)))
        return mem

    nit = cfg["nit"] or NJ
    n0 = (LAG - 1) // U
    nb = (nit - LAG) // U
    assert n0 * U == LAG - 1
    accb[0] = jnp.zeros((2 * SEG, D), F32)
    ob[NJ] = jnp.zeros((2, SEG // 2, D), U32)

    def phase(ph, mem):
        mem = lax.fori_loop(jnp.where(ph == 0, 0, n0), jnp.where(ph == 0, n0, n0 + nb), body, mem)
        pl.when(ph == 0)(routed_mlp)
        return mem

    mem = lax.fori_loop(0, 2, phase, mem1)
    for n in range(U):
        o_copy(nb * U - U + n).start()
    for jp in range(LAG + nb * U, nit):
        mem = step(1, jp, step(0, jp, mem, emit(jp - LAG, jp - LAG)))
    rest = range(nit - LAG, nit - 1)
    step(2, nit - 1, mem, (o for jp in rest for o in emit(jp, jp)))
    for jp in range(nb * U, nit - 1):
        o_copy(jp).start()
    for _ in emit(nit - 1, nit - 1):
        pass
    o_copy(nit - 1).start()
    o_copy(pl.ds(0, nit)).wait()


def make(cfg=None):
    cfg = dict(CFG, **(cfg or {}))

    def fn(A_x, A_mem0, A_Wq, A_Wk, A_Wv, A_Wo, A_seg_len, B_x, B_w_r, B_w_gate, B_w_up, B_w_down, gate_w):
        del B_x
        B, S, D = A_x.shape
        _, H, E = A_Wq.shape
        M = A_mem0.shape[1]
        F = B_w_gate.shape[1]
        SEG = int(A_seg_len)
        assert B == 1 and E == LANES
        NP, DH, NJ = H // 2, D // 2, S // SEG // 2
        P5 = SEG - cfg["R5"]
        any_spec = pl.BlockSpec(memory_space=pl.ANY)
        vmem_spec = pl.BlockSpec(memory_space=pltpu.VMEM)
        out = pl.pallas_call(
            functools.partial(_kernel, S=S, D=D, H=H, M=M, SEG=SEG, cfg=cfg),
            out_shape=jax.ShapeDtypeStruct((NJ, 2, SEG, D), BF16),
            in_specs=[any_spec, vmem_spec, any_spec, any_spec, any_spec, any_spec, vmem_spec,
                      any_spec, any_spec, any_spec, vmem_spec],
            out_specs=any_spec,
            scratch_shapes=[
                *[pltpu.VMEM((NP, DH // 16, 56, LANES), U32)] * 3,
                pltpu.VMEM((NP, 7, E // 2, DH), U32),
                pltpu.VMEM((D // 2, F), U32),
                pltpu.VMEM((D // 2, F), U32),
                pltpu.VMEM((F // 2, D), U32),
                pltpu.VMEM((NJ, 2, SEG // 2, D), U32),
                pltpu.VMEM((NJ + 1, 2, SEG // 2, D), U32),
                pltpu.VMEM((NJ, 2 * SEG, LANES), F32),
                pltpu.VMEM((NJ - 1, SEG // 2, DH), U32),
                pltpu.VMEM((NJ - 1, max(P5, 8), DH), F32),
                *[pltpu.VMEM((NP, (NJ - 1) * SEG, LANES), F32)] * 3,
                *[pltpu.VMEM((NP, max((NJ - 1) * P5, 8), LANES), F32)] * 3,
                pltpu.VMEM((7, M + 2 * SEG, DH), F32),
                pltpu.VMEM((3, NP, 3, SEG, LANES), F32),
                *[pltpu.VMEM((H, SEG, LANES), F32)] * 4,
                pltpu.VMEM((NP, M, 2 * LANES), F32),
                pltpu.VMEM((4, 2 * SEG, NP * LANES), F32),
                pltpu.VMEM((4, M + SEG, NP * LANES), F32),
                pltpu.VMEM((4, 2 * SEG, DH), F32),
                pltpu.VMEM((4, M + SEG, DH), F32),
                pltpu.VMEM((cfg["LAG"], 2 * SEG, D), F32),
                pltpu.VMEM((TOP_C, D), F32),
                pltpu.VMEM((TOP_C, LANES), F32),
                pltpu.SMEM((TOP_C,), jnp.int32),
                pltpu.SemaphoreType.DMA((3,)),
                pltpu.SemaphoreType.DMA((NP,)),
                pltpu.SemaphoreType.DMA((NP // 2,)),
                pltpu.SemaphoreType.DMA((4,)),
                pltpu.SemaphoreType.DMA,
            ],
            compiler_params=pltpu.CompilerParams(vmem_limit_bytes=126 * 1024 * 1024, internal_scratch_in_bytes=48 * 1024, **cfg.get("cp", {})),
            name="gmk",
        )(
            A_x.reshape(NJ, 2, SEG, D), A_mem0.reshape(M, D),
            A_Wq.reshape(D // 16, 16, H, E), A_Wk.reshape(D // 16, 16, H, E), A_Wv.reshape(D // 16, 16, H, E),
            A_Wo.reshape(NP, 2, E, D), B_w_r.reshape(D // LANES, LANES),
            B_w_gate, B_w_up, B_w_down, gate_w.reshape(D // LANES, LANES),
        )
        return out.reshape(B, S, D)

    return fn


pallas_gated_mix__memory_aug_recurrent_mem_tr__moe_arch_mod__prompt_kernel = jax.jit(make(), static_argnames=("A_seg_len",))
```

```python
import functools

import jax
import jax.numpy as jnp
import numpy as np
from jax import lax
import jax.experimental.pallas as pl
import jax.experimental.pallas.tpu as pltpu

F32 = jnp.float32
BF16 = jnp.bfloat16
U32 = jnp.uint32
LANES = 128
TOP_C = 8
HI16 = np.uint32(0xFFFF0000)
LO16 = np.uint32(0x0000FFFF)

CFG = dict(
    R5=32,
    nit=None,
    NC=8,
    GP=2,
    R2=16,
    lead=3,
    ahead=3,
    tail=7,
    near=[[0, 8, 8, 8, 8, 8, 8, 0], [0, 8, 8, 8, 8, 8, 8, 0], [0, 0, 0, 0, 0, 0, 0, 0]],
    pace=[[4, 18], [4, 20]],
    odd=['aaaa aaaa aaaa aaaa aaaa aaaa', 'SaaaaaaaaaaaaVaaaaaaaaaaaa', 'sSnaeaaaaoaoaaaaoasVaaaoaaaaaaaeooa', 'nSaaoaoaaaasaoVaaaaaaaaaaaaSaaaa', 'oomoooosoVssoomsoosomooo'],
    even=['aaaa aaaa aaaa aaaa aaaa aaaa', 'aaaaSaaaaaaaaaaaaVaaaaaaaa', 'sSnaadaoadaoaaaaaosVdaaoaaaoaadaaoa', 'nSadasoaooaaaaaadaaadaVaadaSaaaa', 'omOoooOsVsosooomosooosom'],
    last=('aaaa aaaa aaaa S aaaa', 'aaaa aaaa aaaa VS aaaa', 'oeaoaa oaaoaa oeaoaa VS oaaoaa', 'oaaoaa oaaoaa oaaoaa VS oaaoaa', 'oooVooooo oooooooo'),
    vb=1,
)


def _dot(a, b):
    return jnp.dot(a, b, preferred_element_type=F32)


def _dot_nt(a, b):
    return lax.dot_general(a, b, (((1,), (1,)), ((), ())), preferred_element_type=F32)


def _sigmoid(z):
    return 1.0 / (1.0 + jnp.exp(-z))


def _cat(*xs, axis=0):
    return jnp.concatenate(xs, axis=axis)


def _tile(c):
    return slice(c * LANES, (c + 1) * LANES)


def _tree(op, xs):
    while len(xs) > 1:
        xs = [op(*xs[i:i + 2]) if i + 1 < len(xs) else xs[i] for i in range(0, len(xs), 2)]
    return xs[0]


def _recip(d):
    r = pl.reciprocal(d, approx=True)
    return r * (2.0 - d * r)


def _aligned(i, n):
    return i if isinstance(i, int) else pl.multiple_of(i, n)


def _unpack(u):
    return pltpu.bitcast(u, BF16).astype(F32)


def _pack(x):
    return pltpu.bitcast(x.astype(BF16), U32)


def _kernel(
    x_hbm, mem0_ref, wq_hbm, wk_hbm, wv_hbm, wo_hbm, wr_ref, wg_hbm, wu_hbm, wd_hbm, gw_ref,
    out_hbm,
    wq, wk, wv, wo, wg, wu, wd, xb, gate, big2, big5, p2q, p2k, p2v, p5q, p5k, p5v,
    lq, mid, tq, tk, tv, oa, om, lo_a, lo_b, oacc_a, oacc_b, accb, xsel, ysel, mlp, rsel, idx_ref,
    sem_x, sem_w, sem_wo, sem_m, sem_o,
    *, S, D, H, M, SEG, cfg,
):
    NP = H // 2
    NJ = S // SEG // 2
    DH = D // 2
    ND = D // LANES
    NH = DH // LANES
    R5, AH, NC, TAIL = cfg["R5"], cfg["ahead"], cfg["NC"], cfg["tail"]
    P5 = SEG - R5
    L = M + SEG
    scale = np.float32(LANES ** -0.5)
    tok, wqkv = (tq, tk, tv), (wq, wk, wv)
    pre2, pre5 = (p2q, p2k, p2v), (p5q, p5k, p5v)

    xw = x_hbm.bitcast(U32)
    JC = 4
    NXC = NJ // JC

    def x_even(c):
        pairs = pl.ds(c * JC, JC)
        return pltpu.make_async_copy(xw.at[pairs, 0], xb.at[pairs, 0], sem_x.at[c])

    x_odd = pltpu.make_async_copy(xw.at[:, 1], xb.at[pl.ds(0, NJ), 1], sem_x.at[NXC])

    def w_copies(p):
        return [
            pltpu.make_async_copy(
                w.bitcast(U32).at[pl.ds(half * (DH // 16), DH // 16), :, p, :],
                wqkv[j].at[p, :, pl.ds(half * 16, 16), :], sem_w.at[p])
            for j, w in enumerate((wq_hbm, wk_hbm, wv_hbm)) for half in range(2)]

    PG = 2
    NWO = NP // PG

    def wo_copies(g):
        return [
            pltpu.make_async_copy(
                wo_hbm.bitcast(U32).at[g * PG + n, hh],
                wo.at[g * PG + n, :, pl.ds((1 + 2 * hh) * DH, D)], sem_wo.at[g])
            for n in range(PG) for hh in range(2)]

    def slot(i, cols):
        return slice(i * DH + cols.start, i * DH + cols.stop)

    NF = wg.shape[0] - 1

    FA = 6

    def m_copies(lo, hi):
        sem = sem_m.at[int(lo > 0)]
        return [pltpu.make_async_copy(wd_hbm.bitcast(U32).at[lo:hi], wd.at[lo:hi], sem)] + [
            pltpu.make_async_copy(src.bitcast(U32).at[:, _tile(f)], dst.at[f], sem)
            for f in range(lo, hi) for src, dst in ((wg_hbm, wg), (wu_hbm, wu))]

    def m_wait(lo, hi):
        for w in (wg, wu, wd):
            pltpu.make_async_copy(w.at[lo:hi], w.at[lo:hi], sem_m.at[int(lo > 0)]).wait()

    def o_copy(lo, hi):
        return pltpu.make_async_copy(xb.at[lo:hi], out_hbm.bitcast(U32).at[lo:hi], sem_o)

    def start(copies):
        for c in copies:
            c.start()

    def wait(copies):
        for c in copies:
            c.wait()

    def w_in(j, p, i):
        return pltpu.bitcast(wqkv[j][p, :, 8 * i:8 * i + 8, :].reshape(DH // 2, LANES), BF16)

    def combine_in(j, p, t, after=lambda u: u):
        top, bot = after(wqkv[j][p, t, 0:16, :]), after(wqkv[j][p, t, 16:32, :])
        b11, b12, b21, b22 = (
            pltpu.bitcast(u, F32) for u in (top << 16, top & HI16, bot << 16, bot & HI16))
        for i, w in enumerate((b11 + b22, b11, b12 - b22, b21 - b11, b22, b11 + b12, b21 + b22)):
            wqkv[j][p, t, 8 * i:8 * i + 8, :] = _pack(w)

    def combine_out(p, t, n, after):
        rows, cols = slice(8 * t, 8 * t + 8), slice(2 * n * LANES, (2 * n + 2) * LANES)
        b11, b12, b21, b22 = (_unpack(after(wo[p, rows, slot(i, cols)])) for i in (1, 2, 3, 4))
        for i, w in ((0, b11 + b22), (2, b12 - b22), (3, b21 - b11), (5, b11 + b12), (6, b21 + b22)):
            wo[p, rows, slot(i, cols)] = _pack(w)

    def row_dot(xr, w):
        acc = xr[:, _tile(0)] * w[0:1, :]
        for c in range(1, ND):
            acc = acc + xr[:, _tile(c)] * w[c:c + 1, :]
        return jnp.sum(acc, axis=1, keepdims=True)

    qi = lax.broadcasted_iota(jnp.int32, (L, L), 0)
    ki = lax.broadcasted_iota(jnp.int32, (L, L), 1)
    mask = (qi < M) | (qi >= ki)

    def probs(q, k, msk):
        sc = jnp.where(msk, _dot_nt(q, k.astype(BF16) if cfg.get('kb') else k), -1e9 / scale)
        e = jnp.exp2((sc - jnp.max(sc, axis=1, keepdims=True)) * (scale * LOG2E))
        return e * _recip(jnp.sum(e, axis=1, keepdims=True))

    row = lax.broadcasted_iota(jnp.int32, (8, 1), 0)
    LOG2E = np.float32(np.log2(np.e))

    def near_rows(q, k, v, nb, per, idle):
        qs = (yield)(q()) * (scale * LOG2E)
        sc = []
        for b in range(nb):
            for d0 in range(0, 8, per):
                kb = (yield)(k(b))
                for d in range(d0, d0 + per):
                    z = jnp.sum(qs * (pltpu.roll(kb, d, 0) if d else kb), axis=1, keepdims=True)
                    sc.append(jnp.where(row >= d, z, -1e9 * LOG2E) if d and b == nb - 1 else z)
        top = functools.reduce(jnp.maximum, sc)
        for _ in range(idle):
            yield
        o = total = None
        for b in range(nb):
            for d0 in range(0, 8, per):
                after = yield
                vb, base = after(v(b)), after(top)
                for d in range(d0, d0 + per):
                    e = jnp.exp2(sc[8 * b + d] - base)
                    term = e * (pltpu.roll(vb, d, 0) if d else vb)
                    o, total = (term, e) if o is None else (o + term, total + e)
        return o * _recip(total)

    start([x_even(0), x_odd])
    start(w_copies(0))
    wg[NF] = jnp.zeros(wg.shape[1:], U32)
    wu[NF] = jnp.zeros(wu.shape[1:], U32)
    wd[NF] = jnp.zeros(wd.shape[1:], U32)
    ysel[...] = jnp.zeros_like(ysel)
    accb[0] = jnp.zeros((2 * SEG, D), F32)
    xb[NJ] = jnp.zeros((2, SEG // 2, D), U32)
    wait([x_even(0), x_odd])
    start(w_copies(1))
    for jp in range(1, NJ):
        b = _unpack(xb[jp, 1])
        big2[jp - 1] = _pack(b[:, :DH] + b[:, DH:])
        if P5:
            a = _unpack(xb[jp, 0])[R5:]
            big5[jp - 1] = a[:, :DH] + a[:, DH:]
    h0 = _cat(mem0_ref[...].astype(F32), _unpack(xb[0, 0]), _unpack(xb[0, 1]))
    l0 = M + 2 * SEG
    lq[1, 0:l0, :] = h0[:, :DH] + h0[:, DH:]
    lq[2, 0:l0, :] = h0[:, :DH]
    lq[3, 0:l0, :] = h0[:, DH:]
    lo_b[0, 0:2 * M, 0:DH] = jnp.zeros((2 * M, DH), F32)
    wait(w_copies(0))
    if cfg.get("early", 1):
        start(w_copies(2))
    for j in range(3):
        for t in range(DH // 16):
            combine_in(j, 0, t)

    lane = lax.broadcasted_iota(jnp.int32, (8, LANES), 1)
    sub = lax.broadcasted_iota(jnp.int32, (8, LANES), 0)
    WL = cfg.get("wlead", 3)

    def score_jobs(p, keys):
        g0 = p * (JC * 2 * SEG // 8)
        rc = [jnp.zeros((8, LANES), F32)]

        def job(n, after):
            jp = p * JC + n // 4
            xr = _unpack(after(xb[jp, (n // 2) % 2, (n % 2) * 8:(n % 2) * 8 + 8, :]))
            gate[jp, (n % 4) * 16:(n % 4) * 16 + 16, :] = jnp.broadcast_to(
                _sigmoid(row_dot(xr, gw_ref[...].astype(F32))), (16, LANES))
            r = row_dot(xr, wr_ref[...].astype(F32))
            for i in range(2):
                rc[0] = jnp.where(lane == g0 % LANES + 2 * n + i, r[8 * i:8 * i + 8], rc[0])

        def finish():
            r = rc[0].astype(BF16).astype(F32) + 0.0
            bits = pltpu.bitcast(r, jnp.int32)
            mono = lax.shift_right_logical(jnp.where(bits < 0, ~bits, bits | np.int32(-2 ** 31)), 16)
            mono = jnp.where(r != r, 0, mono)
            new = []
            for vi, old in enumerate(keys):
                grp = vi * LANES + lane
                fresh = pltpu.bitcast(mono * S + (S - 1 - (grp * 8 + sub)) + 0x10000000, F32)
                new.append(jnp.where((grp >= g0) & (grp < g0 + JC * 2 * SEG // 8), fresh, old))
            return tuple(new)

        return [functools.partial(job, n) for n in range(4 * JC)], finish

    def pick_row(n, keys):
        best = functools.reduce(jnp.maximum, keys)
        best = jnp.max(jnp.max(best, axis=1, keepdims=True), axis=0, keepdims=True)
        bi = pltpu.bitcast(jnp.broadcast_to(best, (8, LANES)), jnp.int32)
        mono = lax.shift_right_logical(bi - 0x10000000, int(np.log2(S))) << 16
        score = pltpu.bitcast(jnp.where(mono < 0, mono & np.int32(0x7FFF0000), ~mono & np.int32(-65536)), F32)
        idx = (S - 1) - (bi[0, 0] & (S - 1))
        idx_ref[n] = idx
        rsel[pl.ds(n, 1), :] = score[0:1]
        word = xb[idx // (2 * SEG), (idx // SEG) % 2, pl.ds((idx % SEG) // 2, 1), :]
        xsel[pl.ds(n, 1), :] = pltpu.bitcast(jnp.where(idx % 2 == 0, word << 16, word & HI16), F32)
        return tuple(jnp.where(kv == best, 0.0, kv) for kv in keys)

    def out_jobs(p):
        def product(half, t, after):
            cols = slice(t * 2 * LANES, (t + 1) * 2 * LANES)
            w = pltpu.bitcast(_cat(wo[p, :, slot(1 + half, cols)], wo[p, :, slot(3 + half, cols)]), BF16)
            at = (0, slice(half * M, (half + 1) * M), cols)
            lo_b[at] = lo_b[at] + _dot(om[p], w)

        first = [functools.partial(product, half, t) for t in range(2) for half in range(2)]
        rest = [functools.partial(combine_out, p, t, n) for n in range(NH // 2) for t in range(LANES // 16)]
        return first[:2] + rest[:4] + first[2:3] + rest[4:8] + first[3:] + rest[8:]

    def spread(jobs, lo, hi):
        return [(lo + n * (hi - lo) // len(jobs), job) for n, job in enumerate(jobs)]

    NA = 3 * (4 + NJ - 1)

    def pro_step(p, never, plan, midway=None):
        plan = sorted(plan, key=lambda e: e[0])
        seen = [0]

        def anchor(y):
            def after(u):
                r, c = u.shape
                return jnp.where(never, _cat(*[pltpu.bitcast(y[0:r], U32)] * (c // LANES), axis=1), u)

            while plan and plan[0][0] <= seen[0]:
                plan.pop(0)[1](after)
            seen[0] += 1

        def first(j):
            s = lq[1, 0:l0, :]
            c0 = _dot(s, w_in(j, p, 1)) + _dot(lq[3, 0:l0, :], w_in(j, p, 3))
            c1 = _dot(lq[2, 0:l0, :], w_in(j, p, 2)) + _dot(s, w_in(j, p, 4))
            tok[j][2 * p] = c0[L:]
            tok[j][2 * p + 1] = c1[L:]
            for y in (c0, c0[L:], c1, c1[L:]):
                anchor(y)
            return c0[:L], c1[:L]

        edges = [(NJ - 1) * c // NC for c in range(NC + 1)]

        def bulk(j):
            for c in range(NC):
                lo, hi = edges[c], edges[c + 1]
                lhs = pltpu.bitcast(big2[lo:hi].reshape((hi - lo) * SEG // 2, DH), BF16)
                y = _dot(lhs, w_in(j, p, 1))
                pre2[j][p, lo * SEG:hi * SEG, :] = y
                if P5:
                    pre5[j][p, lo * P5:hi * P5, :] = _dot(big5[lo:hi].reshape((hi - lo) * P5, DH), w_in(j, p, 4))
                for n in range(hi - lo):
                    anchor(y[n * SEG:(n + 1) * SEG])

        q, k, v = first(0), first(1), first(2)
        e = [probs(q[i], k[i], mask) for i in range(2)]
        bulk(0)
        o = [_dot(e[i], v[i]) for i in range(2)]
        oa[2 * p] = o[0][M:]
        oa[2 * p + 1] = o[1][M:]
        om[p] = _cat(o[0][:M], o[1][:M], axis=1)
        if midway:
            midway()
        bulk(1)
        bulk(2)
        assert not plan

    def in_jobs(p):
        return [functools.partial(combine_in, j, p, t) for j in range(3) for t in range(DH // 16)]

    def pro_main(p, keys):
        wait(w_copies(p + 1))
        pl.when(p >= 2)(lambda: x_even(p - 1).wait())
        pl.when(p + 1 < NXC)(lambda: x_even(p + 1).start())
        pl.when(p == 0)(lambda: [start(w_copies(n)) for n in range(2 + cfg.get('early', 1), AH + 1)] and None or None)
        start(w_copies(p + 1 + AH))
        g = p - (NP - TAIL - WL)
        pl.when(g >= 0)(lambda: start(wo_copies(g)))
        jobs, finish = score_jobs(jnp.maximum(p - 1, 0), keys)
        pro_step(p, p < 0, spread(jobs, 0, NA - 12) + spread(in_jobs(p + 1), 0, NA - 1))
        return finish()

    def pro_tail(p, keys):
        g = p - (NP - TAIL)
        wait(w_copies(p + 1))
        pl.when(p + 1 + AH < NP)(lambda: start(w_copies(p + 1 + AH)))
        pl.when(g + WL < NWO)(lambda: start(wo_copies(g + WL)))
        wait(wo_copies(g))
        keys = pick_row(g, keys)
        jobs = [job for n in range(PG) for job in out_jobs(g * PG + n)]
        pro_step(p, p < 0, spread(jobs, 0, NA - 2) + spread(in_jobs(p + 1), 0, NA - 1))
        return keys

    def pro_last(keys):
        for n in range(TAIL - 1, TOP_C):
            keys = pick_row(n, keys)

        def midway():
            for g in range(TAIL - 1, NWO):
                wait(wo_copies(g))
            m_copies(0, FA)[0].start()

        jobs = [job for p in range((TAIL - 1) * PG, NP) for job in out_jobs(p)]
        loads = [lambda after, c=c: c.start() for c in m_copies(0, FA)[1:] + m_copies(FA, NF)[1:]]
        pro_step(NP - 1, idx_ref[0] < 0, spread(jobs, 12 + NJ - 1, NA - 2) + spread(loads, 12 + NJ - 1, NA - 2), midway)

    keys = tuple(jnp.zeros((8, LANES), F32) for _ in range(S // (8 * LANES)))
    if not cfg.get('loop'):
        keys = lax.fori_loop(0, NP - TAIL, pro_main, keys)
        keys = lax.fori_loop(NP - TAIL, NP - 1, pro_tail, keys)
        pro_last(keys)
    m_copies(FA, NF)[0].start()
    mem1 = _cat(lo_b[0, 0:M, 0:DH], lo_b[0, M:2 * M, 0:DH], axis=1)

    def mlp_slice(f):
        pre = []
        for w in (wg, wu):
            for half in range(2):
                rows = slice(half * DH // 2, (half + 1) * DH // 2)
                lanes = slice(half * DH, (half + 1) * DH)
                mlp[len(pre)] = _dot(xsel[:, lanes], pltpu.bitcast(w[f, rows, :], BF16))
                pre.append(mlp[len(pre)])
                yield
        a = pre[0] + pre[1]
        hid = a * _sigmoid(a) * (pre[2] + pre[3])
        for half in range(2):
            lanes = slice(half * DH, (half + 1) * DH)
            ysel[:, lanes] = ysel[:, lanes] + _dot(hid, pltpu.bitcast(wd[f, :, lanes], BF16))
            yield

    def apply_mlp(emitted):
        b = xsel[...] + ysel[...] * _cat(*([_sigmoid(rsel[...])] * ND), axis=1)
        b = b.astype(BF16).astype(F32)
        for i in range(TOP_C):
            idx = idx_ref[i]
            jp, r = idx // (2 * SEG), idx % (2 * SEG)
            g = _cat(*([gate[jp, pl.ds(r, 1), :]] * ND), axis=1)
            a = accb[jnp.minimum(jp, emitted - 1), pl.ds(r, 1), :]
            row = jnp.where(jp < emitted, g * a + (1.0 - g) * b[i:i + 1], b[i:i + 1])
            row = pltpu.bitcast(row.astype(BF16).astype(F32), U32)
            at = (jp, r // SEG, pl.ds((r % SEG) // 2, 1), slice(None))
            word = xb[at]
            xb[at] = jnp.where(idx % 2 == 0, (word & HI16) | (row >> 16), (word & LO16) | row)

    def emit(jp, dst):
        for c in range(ND):
            g = gate[jp]
            b = _cat(_unpack(xb[dst, 0, :, _tile(c)]), _unpack(xb[dst, 1, :, _tile(c)]))
            o = _pack(g * accb[jp, :, _tile(c)] + (1.0 - g) * b)
            xb[dst, 0, :, _tile(c)] = o[:SEG // 2]
            xb[dst, 1, :, _tile(c)] = o[SEG // 2:]
            yield o

    never = idx_ref[0] < 0
    GP = cfg["GP"]
    NG = NP // GP
    NW = 4 // GP
    R2 = cfg["R2"]

    def step(kind, jp, mem, side=iter(()), extra=iter(())):
        a1, a2 = mem[:, :DH], mem[:, DH:]
        if kind != 2:
            xa, xc = _unpack(xb[jp, 0]), _unpack(xb[jp, 1])
            a11, a12, a21, a22 = xa[:, :DH], xa[:, DH:], xc[:, :DH], xc[:, DH:]
        if kind == 0:
            rows = {2: _cat(a1, a11), 3: _cat(a2, a22), 4: _cat(a1 + a2, (a11 + a12)[:R5]) if R5 else a1 + a2,
                    1: a1 + a2}
        elif kind == 1:
            rows = {5: _cat(a1, a21 - a11), 0: _cat(a2, a11 + a22), 6: _cat(a2, a12 - a22), 1: a1 + a2}
        else:
            rows = {2: a1, 3: a2, 4: a1 + a2, 1: a1 + a2}
        for i, r in rows.items():
            lq[i, 0:r.shape[0], :] = r
        slots = list(rows)
        prod, full, ex, acc = {}, {}, {}, {}
        lo = (lo_a, lo_b, lo_a)[kind]
        orows = ({3: L, 2: L, 4: L, 1: M + R2}, {5: L, 0: L, 6: L, 1: L - R2},
                 {2: 2 * SEG, 3: 2 * SEG, 1: 2 * SEG, 4: 2 * SEG})[kind]
        lslot = ({1: 0, 2: 1, 3: 2, 4: 3}, {0: 0, 1: 1, 5: 2, 6: 3}, {1: 0, 2: 1, 3: 2, 4: 0})[kind]

        def proj(j, p, i, anchor=None):
            t = prod.setdefault((j, p), {})
            lhs = lq[i, 0:rows[i].shape[0], :]
            if anchor is not None:
                n = min(anchor.shape[0], lhs.shape[0])
                held = _cat(*[pltpu.bitcast(anchor[r:r + n], F32) for r in range(0, anchor.shape[0], n)], axis=1)
                w = held.shape[1]
                head = _cat(jnp.where(never, held, lhs[:n, :w]), *([lhs[:n, w:]] if w < DH else []), axis=1)
                lhs = _cat(head, lhs[n:]) if n < lhs.shape[0] else head
            t[i] = _dot(lhs, w_in(j, p, i))
            advance(t[i])
            if kind == 0 and i != 1 and rows[i].shape[0] > M:
                mid[j, p, i - 2, 0:rows[i].shape[0] - M, :] = t[i][M:]
            if len(t) < 4:
                return
            if kind == 1:
                at = pl.ds(_aligned((jp - 1) * SEG, SEG), SEG)
                m2, m3, m4, m5 = pre2[j][p, at, :], mid[j, p, 0], mid[j, p, 1], mid[j, p, 2, 0:R5, :]
                if P5:
                    late = pre5[j][p, pl.ds(_aligned((jp - 1) * P5, 8), P5), :]
                    m5 = _cat(m5, late) if R5 else late
                m1, m6, m7 = t[0][M:], t[5][M:], t[6][M:]
                full[j, 2 * p] = _cat(t[1] + (t[6][:M] - t[0][:M]), (m1 + m7) + (m4 - m5))
                full[j, 2 * p + 1] = _cat((t[5][:M] + t[0][:M]) - t[1], m3 + m5)
                tok[j][2 * p] = m2 + m4
                tok[j][2 * p + 1] = (m1 + m6) + (m3 - m2)
            else:
                full[j, 2 * p] = t[1][:M] + t[3][:M]
                full[j, 2 * p + 1] = t[2][:M] + t[4][:M]

        def operand(j, h):
            if kind == 1:
                return full[j, h]
            if kind == 2 and j == 0:
                return tok[j][h]
            return _cat(full[j, h], tok[j][h])

        def near(g):
            return cfg["near"][kind][g]

        def scores(g):
            nr = near(g)
            for h in range(4 * g, 4 * g + 4):
                q, msk = operand(0, h), mask[M:] if kind == 2 else mask
                if nr:
                    q, msk = _cat(q[:M], q[M + nr:]), _cat(msk[:M], msk[M + nr:])
                ex[h] = probs(q, operand(1, h), msk)

        def put_tokens(p, r0, o0, o1):
            t, n = _tile(p), o0.shape[0]
            own, at = slice(r0, r0 + n), slice(M + r0, M + r0 + n)
            if kind == 1:
                oa[2 * p, own] = o0
                oa[2 * p + 1, own] = o1
                return
            a11, a12 = oa[2 * p, own], oa[2 * p + 1, own]
            s2, cut = o0 + o1, min(max(R2 - r0, 0), n)
            if cut:
                lo_a[0, M + r0:M + r0 + cut, t] = s2[:cut]
            if cut < n:
                lo_b[1, M + r0 + cut - R2:M + r0 + n - R2, t] = s2[cut:]
            lo_a[1, at, t] = a11
            lo_a[2, at, t] = o1
            lo_a[3, at, t] = a11 + a12
            lo_b[0, at, t] = a11 + o1
            lo_b[2, at, t] = o0 - a11
            lo_b[3, at, t] = a12 - o1

        def values(g):
            for p in range(2 * g, 2 * g + 2):
                o0, o1 = (_dot(ex.pop(h), operand(2, h).astype(BF16) if cfg.get('vb') else operand(2, h)) for h in (2 * p, 2 * p + 1))
                t = _tile(p)
                if kind == 2:
                    f0, f1 = _cat(oa[2 * p], o0), _cat(oa[2 * p + 1], o1)
                    lo_a[0, :, t] = f0 + f1
                    lo_a[1, :, t] = f0
                    lo_a[2, :, t] = f1
                    continue
                m0, m1 = o0[:M], o1[:M]
                for n, m in enumerate((m0 + m1, m0, m1, m0 + m1) if kind == 0 else (m1, m0 + m1, m0, m1)):
                    lo[n, 0:M, t] = m
                put_tokens(p, near(g), o0[M:], o1[M:])

        nears = [(h, r) for p in range(NP) for r in range(near(p // 2) // 8) for h in (2 * p, 2 * p + 1)]
        close, waiting, running, due = {}, [], [], []

        def near_head(h, r):
            def part(j, b):
                return operand(j, h)[8 * b:8 * b + 8]

            close[h, r] = yield from near_rows(lambda: part(0, 1 + r), functools.partial(part, 1), functools.partial(part, 2), 2 + r, *cfg['pace'][kind])
            if h % 2:
                put_tokens(h // 2, 8 * r, close[h - 1, r], close[h, r])
            due.append(pltpu.bitcast(close[h, r], U32))

        clock = [0]

        def advance(y):
            gap = cfg.get("gap", (99, 99, 99))[kind]
            for r in range(0, y.shape[0], 8):
                clock[0] += 1
                if waiting and (not running or clock[0] >= gap):
                    running.append(waiting.pop(0))
                    clock[0] = 0
                for job in list(running):
                    try:
                        job.send(lambda u: jnp.where(never, y[r:r + 8, 0:LANES], u))
                    except StopIteration:
                        running.remove(job)

        oacc = (oacc_a, oacc_b, oacc_a)[kind]

        def outproj(G, n, i, anchor=None):
            pairs = range(G * GP, (G + 1) * GP)
            cols = slice(n * NW * LANES, (n + 1) * NW * LANES)
            w = pltpu.bitcast(_cat(*[wo[p, :, slot(i, cols)] for p in pairs]), BF16)
            lhs = lo[lslot[i], 0:orows[i], G * GP * LANES:(G + 1) * GP * LANES]
            if anchor is not None:
                head = _cat(jnp.where(never, pltpu.bitcast(anchor[:M], F32), lhs[:M, :LANES]), lhs[:M, LANES:], axis=1)
                lhs = _cat(head, lhs[M:])
            y = _dot(lhs, w)
            advance(y)
            at = (list(orows).index(i), slice(0, orows[i]), cols)
            if G > 0:
                y = y + oacc[at]
            if G < NG - 1 or kind == 0:
                oacc[at] = y
            if G == NG - 1:
                acc[i, n] = y

        NU = NH // NW
        ounits = [(G, n, i) for G in range(NG) for n in range(NU) for i in orows]
        if kind == 0:
            ounits[-4 * NU:] = sorted(ounits[-4 * NU:], key=lambda u: u[2] in (2, 4))
        mats = (1, 2) if kind == 2 else (0, 1, 2)
        units = [(j, p, i) for g in range(NP // 2) for j in mats for p in (2 * g, 2 * g + 1) for i in slots]
        if kind == 1:
            lead = units[0:4 * cfg["lead"]:4]
            units = lead + [u for u in units if u not in lead]
        ready = set()
        quads = {"S": iter(range(NP // 2)), "V": iter(range(NP // 2))}
        for op in cfg["order"][kind].replace(" ", ""):
            if op in "aed":
                proj(*units.pop(0), next(side, None) if op == "e" else due.pop(0) if due and op == "d" else None)
            elif op == "n":
                while nears and nears[0][0] < 4 * ((96 * 2 - len(units)) // 24):
                    waiting.append(near_head(*nears.pop(0)))
                    next(waiting[-1])
            elif op in "osO":
                pick = next(u for u in ounits if kind == 2 or (u[2] == 1) == (op == "s"))
                ounits.remove(pick)
                assert pick[0] in ready and (kind or not near(pick[0]) or (4 * pick[0] + 3, near(pick[0]) // 8 - 1) in close)
                outproj(*pick, due.pop(0) if due and op == 'O' else None)
            elif op == "m":
                next(extra)
            else:
                g = next(quads[op])
                (scores if op == "S" else values)(g)
                if op == 'V':
                    ready.add(g)
        assert not units and not ounits and not nears and not running and not waiting and next(side, None) is None

        def wide(i):
            return _cat(*[acc[i, n] for n in range(NU)], axis=1)

        if kind == 0:
            return _cat(wide(1)[:M] + wide(3)[:M], wide(2)[:M] + wide(4)[:M], axis=1)
        if kind == 1:
            sl = jp - 1
            m4, m3, m5, m2 = oacc_a[0, M:L], oacc_a[1, M:L], oacc_a[2, M:L], oacc_a[3, M:M + R2]
            t1, t6, t7, ts = wide(0), wide(5), wide(6), wide(1)
            if R2 < SEG:
                m2 = _cat(m2, ts[M:])
            accb[sl, 0:SEG, :DH] = (t1[M:] + t7[M:]) + (m4 - m5)
            accb[sl, 0:SEG, DH:] = m3 + m5
            accb[sl, SEG:2 * SEG, :DH] = m2 + m4
            accb[sl, SEG:2 * SEG, DH:] = (t1[M:] + t6[M:]) + (m3 - m2)
            return _cat((ts[:M] - t1[:M]) + t7[:M], t6[:M] - (ts[:M] - t1[:M]), axis=1)
        accb[jp, :, :DH] = wide(1) + wide(3)
        accb[jp, :, DH:] = wide(2) + wide(4)

    nit = cfg["nit"] or NJ

    def finish_mlp():
        apply_mlp(nit - 4)
        o_copy(0, nit - 4).start()

    def body(jp, mem):
        pl.when(jp == 2)(lambda: m_wait(0, FA))
        pl.when(jp == 2 + FA)(lambda: m_wait(FA, NF))
        pl.when(jp == nit - 2)(finish_mlp)
        extra = mlp_slice(jnp.where((jp >= 2) & (jp < 2 + NF), jp - 2, NF))
        mem = step(0, jp, mem, emit(jnp.maximum(jp - 2, 0), jnp.where(jp >= 2, jp - 2, NJ)), extra)
        return step(1, jp, mem, extra=extra)

    mem = lax.fori_loop(1, nit, body, mem1)
    o_copy(nit - 4, nit - 2).start()
    if not cfg.get('loop'):
        step(2, nit - 1, mem, emit(nit - 2, nit - 2))
    else:
        lax.fori_loop(0, 2, lambda i, _: [r.__setitem__(i, r[i + 1]) for r in (tq, tk, tv, oa, wq, wk, wv, p2q, p2k, p2v)] and None, None)
    o_copy(nit - 2, nit - 1).start()
    for _ in emit(nit - 1, nit - 1):
        pass
    o_copy(nit - 1, nit).start()
    o_copy(0, nit).wait()


def make(cfg=None):
    cfg = dict(CFG, **(cfg or {}))
    o, e, l = cfg['odd'], cfg['even'], cfg['last']
    cfg['order'] = (o[0] + o[1] + 5 * o[2] + o[3] + o[4], e[0] + e[1] + 5 * e[2] + e[3] + e[4], l[0] + l[1] + 4 * l[2] + 2 * l[3] + l[4])

    def fn(A_x, A_mem0, A_Wq, A_Wk, A_Wv, A_Wo, A_seg_len, B_x, B_w_r, B_w_gate, B_w_up, B_w_down, gate_w):
        del B_x
        B, S, D = A_x.shape
        _, H, E = A_Wq.shape
        M = A_mem0.shape[1]
        F = B_w_gate.shape[1]
        SEG = int(A_seg_len)
        assert B == 1 and E == LANES
        NP, DH, NJ = H // 2, D // 2, S // SEG // 2
        P5 = SEG - cfg["R5"]
        any_spec = pl.BlockSpec(memory_space=pl.ANY)
        vmem_spec = pl.BlockSpec(memory_space=pltpu.VMEM)
        out = pl.pallas_call(
            functools.partial(_kernel, S=S, D=D, H=H, M=M, SEG=SEG, cfg=cfg),
            out_shape=jax.ShapeDtypeStruct((NJ, 2, SEG, D), BF16),
            in_specs=[any_spec, vmem_spec, any_spec, any_spec, any_spec, any_spec, vmem_spec,
                      any_spec, any_spec, any_spec, vmem_spec],
            out_specs=any_spec,
            scratch_shapes=[
                *[pltpu.VMEM((NP, DH // 16, 56, LANES), U32)] * 3,
                pltpu.VMEM((NP, E // 2, 7 * DH), U32),
                pltpu.VMEM((F // LANES + 1, D // 2, LANES), U32),
                pltpu.VMEM((F // LANES + 1, D // 2, LANES), U32),
                pltpu.VMEM((F // LANES + 1, LANES // 2, D), U32),
                pltpu.VMEM((NJ + 1, 2, SEG // 2, D), U32),
                pltpu.VMEM((NJ, 2 * SEG, LANES), F32),
                pltpu.VMEM((NJ - 1, SEG // 2, DH), U32),
                pltpu.VMEM((NJ - 1, max(P5, 8), DH), F32),
                *[pltpu.VMEM((NP, (NJ - 1) * SEG, LANES), F32)] * 3,
                *[pltpu.VMEM((NP, max((NJ - 1) * P5, 8), LANES), F32)] * 3,
                pltpu.VMEM((7, M + 2 * SEG, DH), F32),
                pltpu.VMEM((3, NP, 3, SEG, LANES), F32),
                *[pltpu.VMEM((H, SEG, LANES), F32)] * 4,
                pltpu.VMEM((NP, M, 2 * LANES), F32),
                pltpu.VMEM((4, 2 * SEG, NP * LANES), F32),
                pltpu.VMEM((4, M + SEG, NP * LANES), F32),
                pltpu.VMEM((4, 2 * SEG, DH), F32),
                pltpu.VMEM((4, M + SEG, DH), F32),
                pltpu.VMEM((NJ, 2 * SEG, D), F32),
                pltpu.VMEM((TOP_C, D), F32),
                pltpu.VMEM((TOP_C, D), F32),
                pltpu.VMEM((4, TOP_C, LANES), F32),
                pltpu.VMEM((TOP_C, LANES), F32),
                pltpu.SMEM((TOP_C,), jnp.int32),
                pltpu.SemaphoreType.DMA((NJ // 4 + 1,)),
                pltpu.SemaphoreType.DMA((NP,)),
                pltpu.SemaphoreType.DMA((NP // 2,)),
                pltpu.SemaphoreType.DMA((2,)),
                pltpu.SemaphoreType.DMA,
            ],
            compiler_params=pltpu.CompilerParams(vmem_limit_bytes=127 * 1024 * 1024, internal_scratch_in_bytes=48 * 1024, **cfg.get("cp", {})),
            name="gmk",
        )(
            A_x.reshape(NJ, 2, SEG, D), A_mem0.reshape(M, D),
            A_Wq.reshape(D // 16, 16, H, E), A_Wk.reshape(D // 16, 16, H, E), A_Wv.reshape(D // 16, 16, H, E),
            A_Wo.reshape(NP, 2, E, D), B_w_r.reshape(D // LANES, LANES),
            B_w_gate, B_w_up, B_w_down.reshape(F // LANES, LANES, D), gate_w.reshape(D // LANES, LANES),
        )
        return out.reshape(B, S, D)

    return fn


pallas_gated_mix__memory_aug_recurrent_mem_tr__moe_arch_mod__prompt_kernel = jax.jit(make(), static_argnames=("A_seg_len",))
```

```python
import functools

import jax
import jax.numpy as jnp
import numpy as np
from jax import lax
import jax.experimental.pallas as pl
import jax.experimental.pallas.tpu as pltpu

F32 = jnp.float32
BF16 = jnp.bfloat16
U32 = jnp.uint32
LANES = 128
TOP_C = 8
HI16 = np.uint32(0xFFFF0000)
LO16 = np.uint32(0x0000FFFF)
LOG2E = np.float32(np.log2(np.e))
MASKED = -1e9

ORDER_ODD = (
    "aaaaaaaaaaaaaaaaaaaaaaaa"
    "SaaaaaaaaaaaaVaaaaaaaaaaaa"
    "sSnaeaaaaoaoaaaaoasVaaaoaaaaaaaeooa"
    "sSnaeaaaaoaoaaaaoasVaaaoaaaaaaaeooa"
    "sSnaeaaaaoaoaaaaoasVaaaoaaaaaaeaooa"
    "sSnaeaaaaoaoaaaaoasVaaaoaaaaaaaeooa"
    "sSnaaaaaoaoaaaaaoasVaaaoaaaaaaaaooa"
    "SnaaoaoaaaasaoVaaaaaaaaaaaaSaaaa"
    "oomoooosoVssoomsoosomooo")
ORDER_EVEN = (
    "aaaaaaaaaaaaaaaaaaaaaaaa"
    "aaaaSaaaaaaaaaaaaVaaaaaaaa"
    "sSnaaaoaddaoaaaaaosVdaaoaaaoaadaaoa"
    "sSnaadaoadaoaaaaaosVdaaoaaaoaaodaaa"
    "sSnaadaoadaoaaaaaosVdaaoaaaaoadaaoa"
    "sSnaadaoadaoaaaaaosVdaaoaaaoaadaaoa"
    "sSnaadaoadoaaaaaaosVdaaoaaaoaadaaoa"
    "nSadasoaoaaoaaaaaaaddaVaadaSaaaa"
    "omoOooOsVssoooomosooosom")
ORDER_LAST = (
    "aaaaaaaaaaaaaSaaa"
    "aaaaaaaaaVaaaaSaaa"
    + 4 * "oeaoaaoaaoaaVeoaaoaSaoaaoa"
    + 2 * "oaaoaaoaaoaaVaoaaoaSaoaaoa"
    + "ooooVoooooooooooo")
ODD, EVEN, LAST = range(3)
NEAR_QUADS = range(1, 7)
NEAR_PAUSE = (18, 20)


def _dot(a, b):
    return jnp.dot(a, b, preferred_element_type=F32)


def _dot_nt(a, b):
    return lax.dot_general(a, b, (((1,), (1,)), ((), ())), preferred_element_type=F32)


def _sigmoid(z):
    return 1.0 / (1.0 + jnp.exp(-z))


def _recip(d):
    r = pl.reciprocal(d, approx=True)
    return r * (2.0 - d * r)


def _cat(*xs, axis=0):
    return jnp.concatenate(xs, axis=axis)


def _tile(c, n=1):
    return slice(c * n * LANES, (c + 1) * n * LANES)


def _bf16(words):
    return pltpu.bitcast(words, BF16)


def _unpack(words):
    return _bf16(words).astype(F32)


def _pack(x):
    return pltpu.bitcast(x.astype(BF16), U32)


def _start(copies):
    for c in copies:
        c.start()


def _wait(copies):
    for c in copies:
        c.wait()


def _spread(jobs, lo, hi):
    return [(lo + n * (hi - lo) // len(jobs), job) for n, job in enumerate(jobs)]


def _kernel(
    x_hbm, mem0_ref, wq_hbm, wk_hbm, wv_hbm, wo_hbm, wr_ref, wg_hbm, wu_hbm, wd_hbm, gw_ref,
    out_hbm,
    wq, wk, wv, wo, wg, wu, wd, xb, gate, big, pre_q, pre_k, pre_v,
    lq, mid, tok_q, tok_k, tok_v, oa, om, lo_a, lo_b, oacc_a, oacc_b, attn,
    xsel, ysel, hidden, rsel, idx_ref,
    sem_x, sem_w, sem_wo, sem_m, sem_o,
    *, S, D, H, M, SEG,
):
    NP = H // 2
    NJ = S // SEG // 2
    DH = D // 2
    ND = D // LANES
    NH = DH // LANES
    L = M + SEG
    scale = np.float32(LANES ** -0.5)
    wqkv, tok, pre = (wq, wk, wv), (tok_q, tok_k, tok_v), (pre_q, pre_k, pre_v)

    JC = 4
    NXC = NJ // JC
    NWO = NP // 2
    NF = wg.shape[0] - 1
    FA = 6
    xw = x_hbm.bitcast(U32)

    def x_even(c):
        pairs = pl.ds(c * JC, JC)
        return pltpu.make_async_copy(xw.at[pairs, 0], xb.at[pairs, 0], sem_x.at[c])

    def w_copies(p, mats):
        return [
            pltpu.make_async_copy(
                (wq_hbm, wk_hbm, wv_hbm)[j].bitcast(U32).at[pl.ds(half * (DH // 16), DH // 16), :, p, :],
                wqkv[j].at[p, :, pl.ds(half * 16, 16), :], sem_w.at[3 * p + j])
            for j in mats for half in range(2)]

    def wo_copies(g):
        return [
            pltpu.make_async_copy(
                wo_hbm.bitcast(U32).at[2 * g + n, head],
                wo.at[2 * g + n, :, pl.ds((1 + 2 * head) * DH, D)], sem_wo.at[g])
            for n in range(2) for head in range(2)]

    def up_copies(f):
        return [
            pltpu.make_async_copy(src.bitcast(U32).at[:, _tile(f)], dst.at[f], sem_m.at[3 * (f >= FA) + n])
            for n, (src, dst) in enumerate(((wg_hbm, wg), (wu_hbm, wu)))]

    def down_copy(lo, hi):
        return pltpu.make_async_copy(wd_hbm.bitcast(U32).at[lo:hi], wd.at[lo:hi], sem_m.at[3 * (lo > 0) + 2])

    def mlp_wait(lo, hi):
        for n, w in enumerate((wg, wu)):
            pltpu.make_async_copy(w.at[lo:hi], w.at[lo:hi], sem_m.at[3 * (lo > 0) + n]).wait()
        down_copy(lo, hi).wait()

    def out_copy(lo, hi):
        return pltpu.make_async_copy(xb.at[lo:hi], out_hbm.bitcast(U32).at[lo:hi], sem_o)

    def w_in(j, p, i):
        return _bf16(wqkv[j][p, :, 8 * i:8 * i + 8, :].reshape(DH // 2, LANES))

    def slot(i, cols):
        return slice(i * DH + cols.start, i * DH + cols.stop)

    def combine_in(j, p, t, after):
        top, bot = after(wqkv[j][p, t, 0:16, :]), after(wqkv[j][p, t, 16:32, :])
        b11, b12, b21, b22 = (
            pltpu.bitcast(u, F32) for u in (top << 16, top & HI16, bot << 16, bot & HI16))
        for i, w in enumerate((b11 + b22, b11, b12 - b22, b21 - b11, b22, b11 + b12, b21 + b22)):
            wqkv[j][p, t, 8 * i:8 * i + 8, :] = _pack(w)

    def combine_out(p, t, n, after):
        rows, cols = slice(8 * t, 8 * t + 8), _tile(n, 2)
        b11, b12, b21, b22 = (_unpack(after(wo[p, rows, slot(i, cols)])) for i in (1, 2, 3, 4))
        for i, w in ((0, b11 + b22), (2, b12 - b22), (3, b21 - b11), (5, b11 + b12), (6, b21 + b22)):
            wo[p, rows, slot(i, cols)] = _pack(w)

    qi = lax.broadcasted_iota(jnp.int32, (L, L), 0)
    ki = lax.broadcasted_iota(jnp.int32, (L, L), 1)
    mask = (qi < M) | (qi >= ki)
    row = lax.broadcasted_iota(jnp.int32, (8, 1), 0)

    def probs(q, k, visible):
        sc = jnp.where(visible, _dot_nt(q, k), MASKED / scale)
        e = jnp.exp2((sc - jnp.max(sc, axis=1, keepdims=True)) * (scale * LOG2E))
        return e * _recip(jnp.sum(e, axis=1, keepdims=True))

    def near_rows(q, k, v, pause):
        qs = (yield)(q()) * (scale * LOG2E)
        sc = []
        for b in range(2):
            for d0 in (0, 4):
                kb = (yield)(k(b))
                for d in range(d0, d0 + 4):
                    z = jnp.sum(qs * (pltpu.roll(kb, d, 0) if d else kb), axis=1, keepdims=True)
                    sc.append(jnp.where(row >= d, z, MASKED * LOG2E) if d and b else z)
        top = functools.reduce(jnp.maximum, sc)
        for _ in range(pause):
            yield
        o = total = None
        for b in range(2):
            for d0 in (0, 4):
                after = yield
                vb, base = after(v(b)), after(top)
                for d in range(d0, d0 + 4):
                    e = jnp.exp2(sc[8 * b + d] - base)
                    term = e * (pltpu.roll(vb, d, 0) if d else vb)
                    o, total = (term, e) if o is None else (o + term, total + e)
        return o * _recip(total)

    lane = lax.broadcasted_iota(jnp.int32, (8, LANES), 1)
    sub = lax.broadcasted_iota(jnp.int32, (8, LANES), 0)
    KEY0 = 0x10000000

    def row_dot(xr, w):
        acc = xr[:, _tile(0)] * w[0:1, :]
        for c in range(1, ND):
            acc = acc + xr[:, _tile(c)] * w[c:c + 1, :]
        return jnp.sum(acc, axis=1, keepdims=True)

    def score_jobs(c, keys):
        groups = JC * 2 * SEG // 8
        g0 = c * groups
        scores = [jnp.zeros((8, LANES), F32)]

        def job(n, after):
            jp = c * JC + n // 4
            xr = _unpack(after(xb[jp, (n // 2) % 2, (n % 2) * 8:(n % 2) * 8 + 8, :]))
            gate[jp, (n % 4) * 16:(n % 4) * 16 + 16, :] = jnp.broadcast_to(
                _sigmoid(row_dot(xr, gw_ref[...].astype(F32))), (16, LANES))
            r = row_dot(xr, wr_ref[...].astype(F32))
            for i in range(2):
                scores[0] = jnp.where(lane == g0 % LANES + 2 * n + i, r[8 * i:8 * i + 8], scores[0])

        def finish():
            r = scores[0].astype(BF16).astype(F32)
            bits = jnp.where(r == 0.0, 0, pltpu.bitcast(r, jnp.int32))
            rank = lax.shift_right_logical(jnp.where(bits < 0, ~bits, bits | np.int32(-2 ** 31)), 16)
            rank = jnp.where(r != r, 0, rank)
            new = []
            for n, old in enumerate(keys):
                group = n * LANES + lane
                key = pltpu.bitcast(rank * S + (S - 1 - (group * 8 + sub)) + KEY0, F32)
                new.append(jnp.where((group >= g0) & (group < g0 + groups), key, old))
            return tuple(new)

        return [functools.partial(job, n) for n in range(4 * JC)], finish

    def word_row(idx):
        return idx // (2 * SEG), (idx // SEG) % 2, pl.ds((idx % SEG) // 2, 1), slice(None)

    def pick_row(n, keys):
        best = functools.reduce(jnp.maximum, keys)
        best = jnp.max(jnp.max(best, axis=1, keepdims=True), axis=0, keepdims=True)
        bits = pltpu.bitcast(jnp.broadcast_to(best, (8, LANES)), jnp.int32)
        rank = lax.shift_right_logical(bits - KEY0, S.bit_length() - 1) << 16
        score = jnp.where(rank < 0, rank & np.int32(0x7FFF0000), ~rank & np.int32(-65536))
        idx = (S - 1) - (bits[0, 0] & (S - 1))
        idx_ref[n] = idx
        rsel[pl.ds(n, 1), :] = pltpu.bitcast(score, F32)[0:1]
        word = xb[word_row(idx)]
        xsel[pl.ds(n, 1), :] = pltpu.bitcast(jnp.where(idx % 2 == 0, word << 16, word & HI16), F32)
        return tuple(jnp.where(key == best, 0.0, key) for key in keys)

    AHEAD = 7
    TAIL = 6
    NC = 8
    NB = 7 + NJ - 1
    NA = 3 * NB

    def needed_by(p):
        return w_copies(p, (1, 2)) + w_copies(p + 1, (0,))

    def queue(lo, hi):
        for p in range(lo, hi):
            _start(needed_by(p))
            if p >= 2:
                x_even(p - 1).start()

    first_x = [x_even(0), pltpu.make_async_copy(xw.at[:, 1], xb.at[pl.ds(0, NJ), 1], sem_x.at[NXC])]
    _start(first_x + w_copies(0, (0,)))
    queue(0, 4)
    wg[NF] = jnp.zeros(wg.shape[1:], U32)
    wu[NF] = jnp.zeros(wu.shape[1:], U32)
    wd[NF] = jnp.zeros(wd.shape[1:], U32)
    ysel[...] = jnp.zeros_like(ysel)
    attn[0] = jnp.zeros((2 * SEG, D), F32)
    xb[NJ] = jnp.zeros((2, SEG // 2, D), U32)
    lo_b[0, 0:2 * M, 0:DH] = jnp.zeros((2 * M, DH), F32)
    _wait(first_x)
    queue(4, AHEAD)
    for jp in range(1, NJ):
        xs = _unpack(xb[jp, 1])
        big[jp - 1] = _pack(xs[:, :DH] + xs[:, DH:])
    a1, a2, a11, a12, a21, a22 = (
        u[:, half * DH:(half + 1) * DH]
        for u in (mem0_ref[...].astype(F32), _unpack(xb[0, 0]), _unpack(xb[0, 1])) for half in range(2))
    rows0 = {2: _cat(a1, a11), 4: _cat(a1 + a2, a11 + a12), 3: _cat(a2, a22), 1: _cat(a1 + a2, a21 + a22),
             0: a11 + a22, 6: a12 - a22, 5: a21 - a11}
    for i, r in rows0.items():
        lq[i, 0:r.shape[0], :] = r
    _wait(w_copies(0, (0,)))
    for t in range(DH // 16):
        combine_in(0, 0, t, lambda u: u)

    def pair_step(p, never, plan):
        plan = sorted(plan, key=lambda entry: entry[0])
        seen = [0]

        def side_work(y):
            def after(u):
                r, c = u.shape
                return jnp.where(never, _cat(*[pltpu.bitcast(y[0:r], U32)] * (c // LANES), axis=1), u)

            while plan and plan[0][0] <= seen[0]:
                plan.pop(0)[1](after)
            seen[0] += 1

        def first(j):
            t = {}
            for i, r in rows0.items():
                t[i] = _dot(lq[i, 0:r.shape[0], :], w_in(j, p, i))
                side_work(t[i])
            m1, m2, m3, m4, m5, m6, m7 = (t[i][-SEG:] for i in range(7))
            tok[j][2 * p] = m2 + m4
            tok[j][2 * p + 1] = (m1 + m6) + (m3 - m2)
            return _cat(t[1][:M] + t[3][:M], (m1 + m7) + (m4 - m5)), t[2] + t[4]

        def bulk(j, chunks):
            for c in chunks:
                lo, hi = (NJ - 1) * c // NC, (NJ - 1) * (c + 1) // NC
                y = _dot(_bf16(big[lo:hi].reshape((hi - lo) * SEG // 2, DH)), w_in(j, p, 1))
                pre[j][p, lo * SEG:hi * SEG, :] = y
                for n in range(hi - lo):
                    side_work(y[n * SEG:(n + 1) * SEG])

        q = first(0)
        bulk(0, range(NC))
        k = first(1)
        bulk(1, range(2))
        e = [probs(q[i], k[i], mask) for i in range(2)]
        bulk(1, range(2, NC))
        v = first(2)
        bulk(2, range(2))
        o = [_dot(e[i], v[i]) for i in range(2)]
        oa[2 * p] = o[0][M:]
        oa[2 * p + 1] = o[1][M:]
        om[p] = _cat(o[0][:M], o[1][:M], axis=1)
        bulk(2, range(2, NC))
        assert not plan

    def in_jobs(j, p, phase):
        jobs = [functools.partial(combine_in, j, p, t) for t in range(DH // 16)]
        return _spread(jobs, phase * NB, (phase + 1) * NB - 6)

    def ahead_jobs(p):
        return in_jobs(1, p, 0) + in_jobs(2, p, 1) + in_jobs(0, p + 1, 2)

    def out_jobs(g):
        def product(p, half, n, after):
            cols = _tile(n, 2)
            w = _bf16(_cat(wo[p, :, slot(1 + half, cols)], wo[p, :, slot(3 + half, cols)]))
            at = (0, slice(half * M, (half + 1) * M), cols)
            lo_b[at] = lo_b[at] + _dot(om[p], w)

        jobs = []
        for p in (2 * g, 2 * g + 1):
            use = [functools.partial(product, p, half, n) for n in range(2) for half in range(2)]
            mix = [functools.partial(combine_out, p, t, n) for n in range(2) for t in range(LANES // 16)]
            jobs += use[:2] + mix[:4] + use[2:3] + mix[4:8] + use[3:] + mix[8:]
        return jobs

    def scoring_step(p, keys):
        _wait(needed_by(p))
        pl.when((p >= 2) & (p <= NXC))(lambda: x_even(p - 1).wait())
        pl.when(p + AHEAD - 1 < NXC)(lambda: x_even(p + AHEAD - 1).start())
        pl.when(p + AHEAD < NP)(lambda: _start(w_copies(p + AHEAD, (1, 2))))
        pl.when(p + AHEAD + 1 < NP)(lambda: _start(w_copies(p + AHEAD + 1, (0,))))
        g = p + AHEAD - (NP - TAIL)
        pl.when(g >= 0)(lambda: _start(wo_copies(g)))
        jobs, finish = score_jobs(jnp.clip(p - 1, 0, NXC - 1), keys)
        pair_step(p, p < 0, _spread(jobs, 0, NA - 12) + ahead_jobs(p))
        return finish()

    def picking_step(p, keys):
        g = p - (NP - TAIL)
        _wait(needed_by(p))
        pl.when(g + AHEAD < NWO)(lambda: _start(wo_copies(g + AHEAD)))
        _wait(wo_copies(g))
        keys = pick_row(g, keys)
        pair_step(p, p < 0, _spread(out_jobs(g), 0, NA - 2) + ahead_jobs(p))
        return keys

    keys = tuple(jnp.zeros((8, LANES), F32) for _ in range(S // (8 * LANES)))
    keys = lax.fori_loop(0, NP - TAIL, scoring_step, keys)
    keys = lax.fori_loop(NP - TAIL, NP - 1, picking_step, keys)
    _wait(w_copies(NP - 1, (1, 2)) + wo_copies(TAIL - 1))
    for n in range(TAIL - 1, TOP_C):
        keys = pick_row(n, keys)
    never = idx_ref[0] < 0
    pair_step(NP - 1, never,
              in_jobs(1, NP - 1, 0) + in_jobs(2, NP - 1, 1) + _spread(out_jobs(TAIL - 1), 0, 2 * NB - 2)
              + [(2 * NB - 1, lambda after: _wait(wo_copies(TAIL)))] + _spread(out_jobs(TAIL), 2 * NB, NA - 1))
    _wait(wo_copies(NWO - 1))
    down_copy(0, FA).start()
    for f in range(NF):
        _start(up_copies(f))
    for job in out_jobs(NWO - 1):
        job(lambda u: u)
    down_copy(FA, NF).start()
    mem1 = _cat(lo_b[0, 0:M, 0:DH], lo_b[0, M:2 * M, 0:DH], axis=1)

    def mlp_slice(f):
        for n, (w, half) in enumerate((w, half) for w in (wg, wu) for half in range(2)):
            hidden[n] = _dot(xsel[:, _tile(half, NH)], _bf16(w[f, half * DH // 2:(half + 1) * DH // 2, :]))
            yield
        a = hidden[0] + hidden[1]
        h = a * _sigmoid(a) * (hidden[2] + hidden[3])
        for half in range(2):
            cols = _tile(half, NH)
            ysel[:, cols] = ysel[:, cols] + _dot(h, _bf16(wd[f, :, cols]))
            yield

    def apply_mlp(mixed):
        b = xsel[...] + ysel[...] * _cat(*[_sigmoid(rsel[...])] * ND, axis=1)
        b = b.astype(BF16).astype(F32)
        for i in range(TOP_C):
            idx = idx_ref[i]
            jp, r = idx // (2 * SEG), idx % (2 * SEG)
            g = _cat(*[gate[jp, pl.ds(r, 1), :]] * ND, axis=1)
            a = attn[jnp.minimum(jp, mixed - 1), pl.ds(r, 1), :]
            new = jnp.where(jp < mixed, g * a + (1.0 - g) * b[i:i + 1], b[i:i + 1])
            new = pltpu.bitcast(new.astype(BF16).astype(F32), U32)
            word = xb[word_row(idx)]
            xb[word_row(idx)] = jnp.where(idx % 2 == 0, (word & HI16) | (new >> 16), (word & LO16) | new)

    def mix(jp, dst, c, a):
        g = gate[jp]
        b = _cat(_unpack(xb[dst, 0, :, _tile(c)]), _unpack(xb[dst, 1, :, _tile(c)]))
        o = _pack(g * a + (1.0 - g) * b)
        xb[dst, 0, :, _tile(c)] = o[:SEG // 2]
        xb[dst, 1, :, _tile(c)] = o[SEG // 2:]
        return o

    def mixes(jp, dst):
        for c in range(ND):
            yield mix(jp, dst, c, attn[jp, :, _tile(c)])

    R2 = SEG // 2

    def step(kind, jp, mem, src=None, side=iter(()), extra=iter(())):
        a1, a2 = mem[:, :DH], mem[:, DH:]
        if kind == LAST:
            rows = {2: a1, 3: a2, 4: a1 + a2, 1: a1 + a2}
        else:
            xa, xc = _unpack(xb[src, 0]), _unpack(xb[src, 1])
            a11, a12, a21, a22 = xa[:, :DH], xa[:, DH:], xc[:, :DH], xc[:, DH:]
            if kind == ODD:
                rows = {2: _cat(a1, a11), 3: _cat(a2, a22), 4: _cat(a1 + a2, a11 + a12), 1: a1 + a2}
            else:
                rows = {5: _cat(a1, a21 - a11), 0: _cat(a2, a11 + a22), 6: _cat(a2, a12 - a22), 1: a1 + a2}
        for i, r in rows.items():
            lq[i, 0:r.shape[0], :] = r
        lo, oacc = ((lo_a, oacc_a), (lo_b, oacc_b), (lo_a, oacc_a))[kind]
        orows = ({3: L, 2: L, 4: L, 1: M + R2}, {5: L, 0: L, 6: L, 1: L - R2},
                 {1: 2 * SEG, 3: 2 * SEG, 2: 2 * SEG, 4: 2 * SEG})[kind]
        lslot = ({1: 0, 2: 1, 3: 2, 4: 3}, {0: 0, 1: 1, 5: 2, 6: 3}, {1: 0, 2: 1, 3: 2, 4: 0})[kind]
        prod, fresh, weights, acc, near_out = {}, {}, {}, {}, {}
        running, due = [], []

        def near(g):
            return 8 if kind != LAST and g in NEAR_QUADS else 0

        def behind(lhs, done):
            if done is None:
                return lhs
            n = min(done.shape[0], lhs.shape[0])
            held = _cat(*[pltpu.bitcast(done[r:r + n], F32) for r in range(0, done.shape[0], n)], axis=1)
            w = held.shape[1]
            head = jnp.where(never, held, lhs[:n, :w])
            head = _cat(head, lhs[:n, w:], axis=1) if w < lhs.shape[1] else head
            return _cat(head, lhs[n:]) if n < lhs.shape[0] else head

        def advance(y):
            for r in range(0, y.shape[0], 8):
                if running:
                    try:
                        running[0].send(lambda u: jnp.where(never, y[r:r + 8, 0:LANES], u))
                    except StopIteration:
                        running.pop(0)

        def project(j, p, i, done):
            t = prod.setdefault((j, p), {})
            t[i] = _dot(behind(lq[i, 0:rows[i].shape[0], :], done), w_in(j, p, i))
            advance(t[i])
            if kind == ODD and i != 1:
                mid[j, p, i - 2] = t[i][M:]
            if len(t) < 4:
                return
            if kind == EVEN:
                m2 = pre[j][p, pl.ds(pl.multiple_of((jp - 1) * SEG, SEG), SEG), :]
                m3, m4, m5 = mid[j, p, 0], mid[j, p, 1], mid[j, p, 2]
                m1, m6, m7 = t[0][M:], t[5][M:], t[6][M:]
                fresh[j, 2 * p] = _cat(t[1] + (t[6][:M] - t[0][:M]), (m1 + m7) + (m4 - m5))
                fresh[j, 2 * p + 1] = _cat((t[5][:M] + t[0][:M]) - t[1], m3 + m5)
                tok[j][2 * p] = m2 + m4
                tok[j][2 * p + 1] = (m1 + m6) + (m3 - m2)
            else:
                fresh[j, 2 * p] = t[1][:M] + t[3][:M]
                fresh[j, 2 * p + 1] = t[2][:M] + t[4][:M]

        def operand(j, h):
            if kind == EVEN:
                return fresh[j, h]
            if kind == LAST and j == 0:
                return tok[j][h]
            return _cat(fresh[j, h], tok[j][h])

        def scores(g):
            for h in range(4 * g, 4 * g + 4):
                q, visible = operand(0, h), mask[M:] if kind == LAST else mask
                if near(g):
                    q, visible = (_cat(u[:M], u[M + near(g):]) for u in (q, visible))
                weights[h] = probs(q, operand(1, h), visible)

        def put_tokens(p, r0, o0, o1):
            t, n = _tile(p), o0.shape[0]
            own, at = slice(r0, r0 + n), slice(M + r0, M + r0 + n)
            if kind == EVEN:
                oa[2 * p, own] = o0
                oa[2 * p + 1, own] = o1
                return
            a11, a12 = oa[2 * p, own], oa[2 * p + 1, own]
            both, cut = o0 + o1, min(R2 - r0, n)
            lo_a[0, M + r0:M + r0 + cut, t] = both[:cut]
            if cut < n:
                lo_b[1, M:M + n - cut, t] = both[cut:]
            lo_a[1, at, t] = a11
            lo_a[2, at, t] = o1
            lo_a[3, at, t] = a11 + a12
            lo_b[0, at, t] = a11 + o1
            lo_b[2, at, t] = o0 - a11
            lo_b[3, at, t] = a12 - o1

        def values(g):
            for p in range(2 * g, 2 * g + 2):
                o0, o1 = (_dot(weights.pop(h), operand(2, h).astype(BF16)) for h in (2 * p, 2 * p + 1))
                if kind == LAST:
                    f0, f1 = _cat(oa[2 * p], o0), _cat(oa[2 * p + 1], o1)
                    for n, f in enumerate((f0 + f1, f0, f1)):
                        lo[n, :, _tile(p)] = f
                    continue
                m0, m1 = o0[:M], o1[:M]
                for n, m in enumerate((m0 + m1, m0, m1, m0 + m1) if kind == ODD else (m1, m0 + m1, m0, m1)):
                    lo[n, 0:M, _tile(p)] = m
                put_tokens(p, near(g), o0[M:], o1[M:])

        def near_head(h):
            def block(j, b):
                return operand(j, h)[8 * b:8 * b + 8]

            near_out[h] = yield from near_rows(
                lambda: block(0, 1), functools.partial(block, 1), functools.partial(block, 2), NEAR_PAUSE[kind])
            if h % 2:
                put_tokens(h // 2, 0, near_out[h - 1], near_out[h])
            due.append(pltpu.bitcast(near_out[h], U32))

        def project_out(g, n, i, done):
            cols = _tile(n, 2)
            w = _bf16(_cat(wo[2 * g, :, slot(i, cols)], wo[2 * g + 1, :, slot(i, cols)]))
            y = _dot(behind(lo[lslot[i], 0:orows[i], _tile(g, 2)], done), w)
            advance(y)
            at = (list(orows).index(i), slice(0, orows[i]), cols)
            if g > 0:
                y = y + oacc[at]
            if g < NP // 2 - 1 or kind == ODD:
                oacc[at] = y
            if g < NP // 2 - 1:
                return
            acc[i, n] = y
            for half, both in enumerate(((1, 3), (2, 4))):
                if kind == LAST and i in both and all((u, n) in acc for u in both):
                    a = acc[both[0], n] + acc[both[1], n]
                    for c in range(2):
                        mix(jp, jp, half * NH + 2 * n + c, a[:, _tile(c)])

        quads = range(NP // 2)
        units = [(j, p, i) for g in quads for j in range(kind == LAST, 3) for p in (2 * g, 2 * g + 1) for i in rows]
        per_quad = len(units) // len(quads)
        outs = [(g, n, i) for g in quads for n in range(2) for i in orows]
        if kind == ODD:
            outs[-8:] = sorted(outs[-8:], key=lambda u: u[2] in (2, 4))
        if kind == EVEN:
            units = units[0:12:4] + [u for u in units if u not in units[0:12:4]]
        nears = [h for h in range(H) if near(h // 4)]
        scored = valued = 0
        for op in (ORDER_ODD, ORDER_EVEN, ORDER_LAST)[kind]:
            done = next(side) if op == "e" else due.pop(0) if op in "dO" and due else None
            if op in "aed":
                project(*units.pop(0), done)
            elif op in "osO":
                g, n, i = next(u for u in outs if kind == LAST or (u[2] == 1) == (op == "s"))
                assert g < valued and (kind != ODD or not near(g) or 4 * g + 3 in near_out)
                outs.remove((g, n, i))
                project_out(g, n, i, done)
            elif op == "S":
                scores(scored)
                scored += 1
            elif op == "V":
                values(valued)
                valued += 1
            elif op == "m":
                next(extra)
            else:
                while nears and nears[0] // 4 < len(quads) + len(units) // -per_quad:
                    running.append(near_head(nears.pop(0)))
                    next(running[-1])
        assert not (units or outs or nears or running) and next(side, None) is None
        if kind == LAST:
            return None
        t = {i: _cat(acc[i, 0], acc[i, 1], axis=1) for i in orows}
        if kind == ODD:
            return _cat(t[1][:M] + t[3][:M], t[2][:M] + t[4][:M], axis=1)
        m4, m3, m5 = oacc_a[0, M:L], oacc_a[1, M:L], oacc_a[2, M:L]
        m2 = _cat(oacc_a[3, M:M + R2], t[1][M:])
        attn[jp - 1, 0:SEG, :DH] = (t[0][M:] + t[6][M:]) + (m4 - m5)
        attn[jp - 1, 0:SEG, DH:] = m3 + m5
        attn[jp - 1, SEG:2 * SEG, :DH] = m2 + m4
        attn[jp - 1, SEG:2 * SEG, DH:] = (t[0][M:] + t[5][M:]) + (m3 - m2)
        shared = t[1][:M] - t[0][:M]
        return _cat(shared + t[6][:M], t[5][:M] - shared, axis=1)

    def finish_mlp():
        xb[NJ:NJ + 2] = xb[NJ - 2:NJ]
        apply_mlp(NJ - 4)
        out_copy(0, NJ - 4).start()

    def two_steps(jp, mem):
        pl.when(jp == 2)(lambda: mlp_wait(0, FA))
        pl.when(jp == 2 + FA)(lambda: mlp_wait(FA, NF))
        pl.when(jp == NJ - 2)(finish_mlp)
        extra = mlp_slice(jnp.where((jp >= 2) & (jp < 2 + NF), jp - 2, NF))
        src = jnp.where(jp >= NJ - 2, jp + 2, jp)
        side = mixes(jnp.maximum(jp - 2, 0), jnp.where(jp >= 2, jp - 2, NJ))
        mem = step(ODD, jp, mem, src, side, extra)
        return step(EVEN, jp, mem, src, extra=extra)

    assert 2 + NF <= NJ - 2
    mem = lax.fori_loop(1, NJ, two_steps, mem1)
    out_copy(NJ - 4, NJ - 2).start()
    step(LAST, NJ - 1, mem, side=mixes(NJ - 2, NJ - 2))
    out_copy(NJ - 2, NJ).start()
    out_copy(0, NJ).wait()


@functools.partial(jax.jit, static_argnames=("A_seg_len",))
def pallas_gated_mix__memory_aug_recurrent_mem_tr__moe_arch_mod__prompt_kernel(
    A_x, A_mem0, A_Wq, A_Wk, A_Wv, A_Wo, A_seg_len, B_x, B_w_r, B_w_gate, B_w_up, B_w_down, gate_w,
):
    del B_x
    B, S, D = A_x.shape
    _, H, E = A_Wq.shape
    M = A_mem0.shape[1]
    F = B_w_gate.shape[1]
    SEG = int(A_seg_len)
    assert (B, S, D, H, E, M, SEG) == (1, 2048, 1024, 32, LANES, 8, 32) and F % LANES == 0
    NP, DH, NJ, NF = H // 2, D // 2, S // SEG // 2, F // LANES
    in_hbm = pl.BlockSpec(memory_space=pl.ANY)
    in_vmem = pl.BlockSpec(memory_space=pltpu.VMEM)
    out = pl.pallas_call(
        functools.partial(_kernel, S=S, D=D, H=H, M=M, SEG=SEG),
        out_shape=jax.ShapeDtypeStruct((NJ, 2, SEG, D), BF16),
        in_specs=[in_hbm, in_vmem, in_hbm, in_hbm, in_hbm, in_hbm, in_vmem, in_hbm, in_hbm, in_hbm, in_vmem],
        out_specs=in_hbm,
        scratch_shapes=[
            *[pltpu.VMEM((NP, DH // 16, 7 * 8, LANES), U32)] * 3,
            pltpu.VMEM((NP, E // 2, 7 * DH), U32),
            *[pltpu.VMEM((NF + 1, D // 2, LANES), U32)] * 2,
            pltpu.VMEM((NF + 1, LANES // 2, D), U32),
            pltpu.VMEM((NJ + 2, 2, SEG // 2, D), U32),
            pltpu.VMEM((NJ, 2 * SEG, LANES), F32),
            pltpu.VMEM((NJ - 1, SEG // 2, DH), U32),
            *[pltpu.VMEM((NP, (NJ - 1) * SEG, LANES), F32)] * 3,
            pltpu.VMEM((7, M + SEG, DH), F32),
            pltpu.VMEM((3, NP, 3, SEG, LANES), F32),
            *[pltpu.VMEM((H, SEG, LANES), F32)] * 4,
            pltpu.VMEM((NP, M, 2 * LANES), F32),
            pltpu.VMEM((4, 2 * SEG, NP * LANES), F32),
            pltpu.VMEM((4, M + SEG, NP * LANES), F32),
            pltpu.VMEM((4, 2 * SEG, DH), F32),
            pltpu.VMEM((4, M + SEG, DH), F32),
            pltpu.VMEM((NJ, 2 * SEG, D), F32),
            *[pltpu.VMEM((TOP_C, D), F32)] * 2,
            pltpu.VMEM((4, TOP_C, LANES), F32),
            pltpu.VMEM((TOP_C, LANES), F32),
            pltpu.SMEM((TOP_C,), jnp.int32),
            pltpu.SemaphoreType.DMA((NJ // 4 + 1,)),
            pltpu.SemaphoreType.DMA((3 * NP,)),
            pltpu.SemaphoreType.DMA((NP // 2,)),
            pltpu.SemaphoreType.DMA((6,)),
            pltpu.SemaphoreType.DMA,
        ],
        compiler_params=pltpu.CompilerParams(
            vmem_limit_bytes=126 * 1024 * 1024, internal_scratch_in_bytes=48 * 1024),
        name="gmk",
    )(
        A_x.reshape(NJ, 2, SEG, D), A_mem0.reshape(M, D),
        A_Wq.reshape(D // 16, 16, H, E), A_Wk.reshape(D // 16, 16, H, E), A_Wv.reshape(D // 16, 16, H, E),
        A_Wo.reshape(NP, 2, E, D), B_w_r.reshape(D // LANES, LANES),
        B_w_gate, B_w_up, B_w_down.reshape(NF, LANES, D), gate_w.reshape(D // LANES, LANES),
    )
    return out.reshape(B, S, D)
```
